```python
import os as _os
_os.environ.setdefault('JAX_PLATFORMS', 'cpu')
import jax
import jax.numpy as jnp

def _softmax(x, axis=-1):
    return jax.nn.softmax(x, axis=axis)

def _gelu(x):
    return jax.nn.gelu(x, approximate=True)

def _silu(x):
    return jax.nn.silu(x)

def _sigmoid(x):
    return jax.nn.sigmoid(x)

def _layernorm(x, axis=-1, eps=1e-05):
    m = jnp.mean(x, axis=axis, keepdims=True)
    v = jnp.var(x, axis=axis, keepdims=True)
    return (x - m) / jnp.sqrt(v + eps)

def _scatter_add(tgt, idx, src, axis=0):
    return tgt.at[idx].add(src)

def _segment_sum(src, seg, n):
    return jax.ops.segment_sum(src, seg, n)

class _Rng:

    def __init__(self, key):
        self._k = key

    def _next(self):
        self._k, sub = jax.random.split(self._k)
        return sub

    def normal(self, shape):
        return jax.random.normal(self._next(), shape, dtype=jnp.bfloat16)

    def randint(self, lo, hi, shape):
        return jax.random.randint(self._next(), shape, lo, hi, dtype=jnp.int32)

    def uniform(self, shape, lo=0.0, hi=1.0):
        return jax.random.uniform(self._next(), shape, jnp.bfloat16, lo, hi)

    def permutation(self, n):
        return jax.random.permutation(self._next(), n)
kernel_name = 'standalone__conformer_family_e_branchformer__speech'

def setup_inputs():
    _rng = _Rng(jax.random.key(int.from_bytes(__import__("os").urandom(4), "little")))
    _w = lambda a: (lambda t: t.astype(jnp.bfloat16) if jnp.issubdtype(t.dtype, jnp.floating) else t)(jnp.asarray(a))
    B, T, D, K = (2, 4000, 256, 31)
    return {'x': _w((lambda *s: _rng.normal(s) * 0.05)(B, T, D)), 'w_qkv': _w((lambda *s: _rng.normal(s) * 0.05)(D, 3 * D)), 'w_att_out': _w((lambda *s: _rng.normal(s) * 0.05)(D, D)), 'w_mlp_in': _w((lambda *s: _rng.normal(s) * 0.05)(D, 2 * D)), 'dw_csgu': _w((lambda *s: _rng.normal(s) * 0.05)(K, D)), 'w_mlp_out': _w((lambda *s: _rng.normal(s) * 0.05)(D, D)), 'dw_merge': _w((lambda *s: _rng.normal(s) * 0.05)(K, 2 * D)), 'w_merge': _w((lambda *s: _rng.normal(s) * 0.05)(2 * D, D))}

def reference(x, w_qkv, w_att_out, w_mlp_in, dw_csgu, w_mlp_out, dw_merge, w_merge):
    B, T, D = x.shape
    K = dw_csgu.shape[0]
    pad = K // 2
    xa = _layernorm(x, axis=-1)
    qkv = jnp.einsum('btd,de->bte', xa, w_qkv)
    q, k, v = (qkv[..., :D].copy(), qkv[..., D:2 * D].copy(), qkv[..., 2 * D:].copy())
    scores = jnp.einsum('btd,bsd->bts', q, k) * D ** (-0.5)
    p = _softmax(scores, axis=-1)
    attn = jnp.einsum('bts,bsd->btd', p, v)
    glob = jnp.einsum('btd,de->bte', attn, w_att_out)
    xc = _layernorm(x, axis=-1)
    h = _gelu(jnp.einsum('btd,de->bte', xc, w_mlp_in))
    u, g = (h[..., :D].copy(), h[..., D:].copy())
    g = _layernorm(g, axis=-1)
    gp = jnp.pad(g, ((0, 0), (pad, pad), (0, 0)))
    gc = jnp.zeros_like(g)
    for i in range(K):
        gc = gc + gp[:, i:i + T, :] * dw_csgu[i][None, None, :]
    loc = jnp.einsum('btd,de->bte', u * gc, w_mlp_out)
    m = jnp.concatenate([glob, loc], axis=-1)
    mp = jnp.pad(m, ((0, 0), (pad, pad), (0, 0)))
    mc = jnp.zeros_like(m)
    for i in range(K):
        mc = mc + mp[:, i:i + T, :] * dw_merge[i][None, None, :]
    m = m + mc
    return x + jnp.einsum('btc,cd->btd', m, w_merge)
```

```python
import functools
import math

import jax
import jax.numpy as jnp
import jax.experimental.pallas as pl
import jax.experimental.pallas.tpu as pltpu

F32 = jnp.float32
BF16 = jnp.bfloat16
U32 = jnp.uint32

B, T, D, KT = 2, 4000, 256, 31
HALO = KT // 2
BQ = 400
NQ = T // BQ
NS = B * NQ
TKP = 4096
SUB = 512
NSUB = TKP // SUB
G = 16
NP = BQ // G
EPS = 1e-5
NEG = -1e30
LOG2E = math.log2(math.e)
GELU_C = math.sqrt(2.0 / math.pi)
CFG = {}
QLINK = CFG.get("QLINK", 2)
PLINK = CFG.get("PLINK", 1)
PHALF = CFG.get("PHALF", 1)
QK_G = CFG.get("QK_G", [8, 16, 28, 36, 44, 52, 60, 68])
MID_G = CFG.get("MID_G", 84)
PV_G = CFG.get("PV_G", [92, 100, 110, 118, 126, 134, 142, 150])
LOC_AT = CFG.get("LOC_AT", 1)
LN_AT = CFG.get("LN_AT", 4)


def _cat(ref, r0, n, tiles):
    return jnp.concatenate([ref[t, pl.ds(r0, n), :] for t in tiles], axis=1)


def _ln(v):
    mu = jnp.mean(v, axis=-1, keepdims=True)
    c = v - mu
    var = jnp.mean(c * c, axis=-1, keepdims=True)
    return c * jax.lax.rsqrt(var + EPS)


def _kernel(x_hbm, wqkv_hbm, wao_hbm, win_hbm, dwc_hbm, wout_hbm, dwm_hbm, wmg_hbm,
            out_hbm,
            wqkv_ref, wao_ref, win_ref, dwc_ref, wout_ref, dwm_ref, wmg_ref,
            x_ref, xl_ref, kv0_ref, kv1_ref, s_ref, acc_ref, q_ref,
            gwin_ref, ghead_ref, u_ref, gm_ref, gm0_ref, lm_ref, lm0_ref,
            cw_ref, wa_ref, wvo_ref, ugc_ref, mc_ref, stage_ref,
            sem_w, sem_x, sem_out):
    kv_refs = (kv0_ref, kv1_ref)

    def x_copy(c):
        r0 = c * BQ if isinstance(c, int) else pl.multiple_of(c * BQ, 16)
        return pltpu.make_async_copy(x_hbm.at[pl.ds(r0, BQ), :], x_ref.at[pl.ds(r0 + 16, BQ), :], sem_x.at[c])

    w_pairs = [(wqkv_hbm, wqkv_ref), (wao_hbm, wao_ref), (dwc_hbm, dwc_ref), (dwm_hbm, dwm_ref),
               (win_hbm, win_ref), (wout_hbm, wout_ref), (wmg_hbm, wmg_ref)]
    w_copies = [pltpu.make_async_copy(src, dst, sem_w.at[i]) for i, (src, dst) in enumerate(w_pairs)]
    for c in w_copies[:4]:
        c.start()
    for c in range(NQ):
        x_copy(c).start()
    for c in w_copies[4:]:
        c.start()
    for c in range(NQ, NS):
        x_copy(c).start()

    x_ref[pl.ds(0, 16), :] = jnp.zeros((16, D), BF16)
    for ct in range(2):
        gwin_ref[ct, pl.ds(0, 16), :] = jnp.zeros((16, 128), F32)
        for r in (gm_ref, lm_ref):
            r[ct] = jnp.zeros((BQ + 32, 128), F32)
        for r in (gm0_ref, lm0_ref):
            r[ct] = jnp.zeros((48, 128), F32)
        xl_ref[ct, pl.ds(B * T, 16), :] = jnp.zeros((16, 128), BF16)
    for kv in kv_refs:
        for ct in range(3):
            kv[ct, pl.ds(T, TKP - T), :] = jnp.zeros((TKP - T, 128), BF16)
    acc_ref[...] = jnp.ones((BQ, D), F32)

    w_copies[0].wait()
    w_copies[1].wait()
    wq = wqkv_ref[:, 0:D]
    wk = wqkv_ref[:, D:2 * D]
    wv = wqkv_ref[:, 2 * D:3 * D]
    a = jax.lax.dot_general(wq, wk, (((1,), (1,)), ((), ())), preferred_element_type=F32)
    wa_ref[...] = (a * (D ** -0.5 * LOG2E)).astype(BF16)
    wvo = jnp.dot(wv, wao_ref[...], preferred_element_type=F32)
    wvo_ref[...] = (wvo - wvo[D - 1:D, :]).astype(BF16)

    w_copies[2].wait()
    w_copies[3].wait()
    dwm = dwm_ref[...].astype(F32)
    dwc = dwc_ref[...].astype(F32)
    for k in range(KT):
        for ct in range(4):
            w = dwm[k:k + 1, ct * 128:(ct + 1) * 128]
            if k == HALO:
                w = w + 1.0
            cw_ref[ct, k] = jnp.broadcast_to(w, (8, 128))
        for ct in range(2):
            cw_ref[4 + ct, k] = jnp.broadcast_to(dwc[k:k + 1, ct * 128:(ct + 1) * 128], (8, 128))

    def ln_chunk(b, i):
        r0 = pl.multiple_of(i * BQ, 16)
        xa = _ln(x_ref[pl.ds(b * T + r0 + 16, BQ), :].astype(F32))
        lo = xa[:, :128].astype(BF16)
        hi = xa[:, 128:].astype(BF16)
        col = jax.lax.broadcasted_iota(jnp.int32, (BQ, 128), 1)
        kv = kv_refs[b]
        kv[0, pl.ds(r0, BQ), :] = lo
        kv[1, pl.ds(r0, BQ), :] = hi
        kv[2, pl.ds(r0, BQ), :] = jnp.where(col == 127, 1.0, xa[:, 128:]).astype(BF16)
        xl_ref[0, pl.ds(b * T + r0, BQ), :] = lo
        xl_ref[1, pl.ds(b * T + r0, BQ), :] = hi

    def ln_body(c, carry):
        x_copy(c).wait()
        ln_chunk(0, c)
        return carry
    jax.lax.fori_loop(0, NQ, ln_body, 0)

    def local_in(r0, n):
        h = jnp.dot(_cat(xl_ref, r0, n, (0, 1)), win_ref[...], preferred_element_type=F32)
        h = 0.5 * h * (1.0 + jnp.tanh(GELU_C * (h + 0.044715 * (h * h * h))))
        return h[:, :D], _ln(h[:, D:])

    def q_proj(r0):
        q = jnp.dot(_cat(xl_ref, r0, BQ, (0, 1)), wa_ref[...], preferred_element_type=F32).astype(BF16)
        q_ref[...] = pltpu.bitcast(q, U32)

    for c in w_copies[4:]:
        c.wait()
    u0, g0 = local_in(0, BQ + 16)
    for ct in range(2):
        u_ref[ct] = u0[:, ct * 128:(ct + 1) * 128]
        gwin_ref[ct, pl.ds(16, BQ + 16), :] = g0[:, ct * 128:(ct + 1) * 128]
        ghead_ref[ct] = g0[BQ:, ct * 128:(ct + 1) * 128]
    q_proj(0)

    def conv_piece(src_ref, st, wt, p0, link):
        acc = None
        for k in range(KT):
            wk_ = cw_ref[wt, k]
            wk_ = jnp.concatenate([wk_] * (G // 8), axis=0)
            t = src_ref[st, pl.ds(p0 + (k - HALO), G), :] * wk_
            if acc is None:
                acc = t if link is None else jnp.where(link[0], link[1], t)
            else:
                acc = acc + t
        return acc

    def out_copy(slot, src0, dst0, n):
        return pltpu.make_async_copy(stage_ref.at[slot, pl.ds(src0, n), :],
                                     out_hbm.at[pl.ds(dst0, n), :], sem_out.at[slot])

    def normalized():
        acc = acc_ref[...]
        return (acc * (1.0 / acc[:, D - 1:D])).astype(BF16)

    def push_block(win, win0, val, joined):
        for ct in range(2):
            new = val[:, ct * 128:(ct + 1) * 128]
            win0[ct, pl.ds(0, 32), :] = win[ct, pl.ds(BQ - 16, 32), :]
            win[ct, pl.ds(0, 16), :] = jnp.where(joined, win[ct, pl.ds(BQ, 16), :], 0.0)
            win[ct, pl.ds(16, BQ), :] = new
            win0[ct, pl.ds(32, 16), :] = jnp.where(joined, new[:16], 0.0)

    def step(b, i, carry):
        s = b * NQ + (i % NQ)
        it = b * NQ * CFG.get('REP', 1) + i
        kv = kv_refs[b]
        negs = -(jax.lax.broadcasted_iota(jnp.int32, (8, 128), 0) + s) - 1
        slot = s % 2

        def never(rows):
            return jnp.concatenate([negs] * (rows // 8), axis=0) >= 0

        if b == 0:
            @pl.when(i < NQ)
            def _():
                x_copy(NQ + i).wait()

        @pl.when(it >= 4)
        def _():
            out_copy(slot, 0, 0, BQ).wait()

        xr0 = pl.multiple_of((jnp.maximum(s, 1) - 1) * BQ, 16)
        sn = jnp.minimum(s + 1, NS - 1)
        rown = pl.multiple_of(sn * BQ, 16)

        state = {"prev": None}
        never_g = never(G)

        def chain(src_ref, st, wt, p0):
            link = None if state["prev"] is None else (never_g, state["prev"])
            acc = conv_piece(src_ref, st, wt, p0, link)
            state["prev"] = acc
            return acc

        def m_piece(ct, j):
            if j == 0:
                acc = chain(gm0_ref if ct < 2 else lm0_ref, ct % 2, ct, 16)
            else:
                acc = chain(gm_ref if ct < 2 else lm_ref, ct % 2, ct, j * G)
            mc_ref[ct, pl.ds(j * G, G), :] = acc.astype(BF16)

        def g_piece(ct, j):
            acc = chain(gwin_ref, ct, 4 + ct, 16 + j * G)
            ugc_ref[ct, pl.ds(j * G, G), :] = (acc * u_ref[ct, pl.ds(j * G, G), :]).astype(BF16)

        pieces = [(g_piece, ct, j) for ct in range(2) for j in range(NP)]
        pieces += [(m_piece, ct, j) for ct in (2, 3, 0, 1) for j in range(NP)]
        done = [0]

        def run_until(n):
            while pieces and done[0] < n:
                f, ct, j = pieces.pop(0)
                f(ct, j)
                done[0] += 1

        qu = q_ref[...]
        mms = []
        for sb in range(NSUB):
            if sb >= QLINK:
                nv = never(BQ // 2)
                mu = pltpu.bitcast(mms[sb - QLINK], U32)
                qs = jnp.concatenate([jnp.where(nv, mu[:BQ // 2], qu[:, :128]),
                                      jnp.where(nv, mu[BQ // 2:], qu[:, 128:])], axis=1)
            else:
                qs = qu
            kc = _cat(kv, sb * SUB, SUB, (0, 1))
            sc = jax.lax.dot_general(pltpu.bitcast(qs, BF16), kc, (((1,), (1,)), ((), ())),
                                     preferred_element_type=F32)
            if sb == NSUB - 1:
                nvalid = T - (TKP - 128)
                col = jax.lax.broadcasted_iota(jnp.int32, (BQ, 128), 1)
                last = jnp.where(col < nvalid, sc[:, SUB - 128:], NEG)
                sc = jnp.concatenate([sc[:, :SUB - 128], last], axis=1)
            s_ref[:, sb * SUB:(sb + 1) * SUB] = sc
            mm = sc[:, 0:128] if sb == 0 else jnp.maximum(mms[-1], sc[:, 0:128])
            for t in range(1, SUB // 128):
                mm = jnp.maximum(mm, sc[:, t * 128:(t + 1) * 128])
            mms.append(mm)
            if sb == 1:
                glob = jnp.dot(normalized(), wvo_ref[...], preferred_element_type=F32)
                push_block(gm_ref, gm0_ref, glob, s % NQ != 1)
            run_until(QK_G[sb])
        mx = jnp.broadcast_to(jnp.max(mms[-1], axis=1, keepdims=True), (BQ, 128))

        u, g = local_in(rown + 16, BQ)
        for ct in range(2):
            gt = g[:, ct * 128:(ct + 1) * 128]
            u_ref[ct, pl.ds(0, 16), :] = u_ref[ct, pl.ds(BQ, 16), :]
            u_ref[ct, pl.ds(16, BQ), :] = u[:, ct * 128:(ct + 1) * 128]
            gwin_ref[ct, pl.ds(0, 16), :] = jnp.where(sn % NQ != 0, gwin_ref[ct, pl.ds(BQ, 16), :], 0.0)
            gwin_ref[ct, pl.ds(16, 16), :] = ghead_ref[ct]
            gwin_ref[ct, pl.ds(32, BQ - 16), :] = gt[:BQ - 16]
            gwin_ref[ct, pl.ds(BQ + 16, 16), :] = jnp.where(sn % NQ != NQ - 1, gt[BQ - 16:], 0.0)
            ghead_ref[ct] = gt[BQ - 16:]
        q_proj(rown)
        run_until(MID_G)

        pvs = []
        for sb in range(NSUB):
            mxs = mx
            if sb >= PLINK:
                mxs = jnp.where(never(BQ), pvs[sb - PLINK], mxs)
            p = jnp.exp2(s_ref[:, sb * SUB:(sb + 1) * SUB] - jnp.concatenate([mxs] * (SUB // 128), axis=1))
            kc = _cat(kv, sb * SUB, SUB, (0, 2))
            pv = jnp.dot(p.astype(BF16), kc, preferred_element_type=F32)
            pvs.append(pv[:, PHALF * 128:(PHALF + 1) * 128])
            if sb == 0:
                acc_ref[...] = pv
            else:
                acc_ref[...] += pv
            run_until(PV_G[sb])
            if sb == LOC_AT:
                assert done[0] >= 4 * NP
                loc = jnp.dot(_cat(ugc_ref, 0, BQ, (0, 1)), wout_ref[...], preferred_element_type=F32)
                push_block(lm_ref, lm0_ref, loc, s % NQ != 0)
            if sb == LN_AT and b + 1 < B:
                ln_chunk(b + 1, i % NQ)
        run_until(1000)

        mo = jnp.dot(_cat(mc_ref, 0, BQ, (0, 1, 2, 3)), wmg_ref[...], preferred_element_type=F32)
        stage_ref[slot] = (x_ref[pl.ds(xr0, BQ), :].astype(F32) + mo).astype(BF16)

        if b == 0:
            @pl.when(it == 1)
            def _():
                c = out_copy(slot, 16, 0, BQ - 16)
                c.start()
                c.wait()

        @pl.when(it >= 2)
        def _():
            out_copy(slot, 0, pl.multiple_of(jnp.maximum(xr0 - 16, 0), 16), BQ).start()

        return carry

    for b in range(B):
        jax.lax.fori_loop(0, NQ * CFG.get('REP', 1), functools.partial(step, b), 0)

    glob = jnp.dot(normalized(), wvo_ref[...], preferred_element_type=F32)
    push_block(gm_ref, gm0_ref, glob, True)
    for ct in (2, 3, 0, 1):
        for j in range(NP + 1):
            if j == 0:
                acc = conv_piece(gm0_ref if ct < 2 else lm0_ref, ct % 2, ct, 16, None)
            else:
                acc = conv_piece(gm_ref if ct < 2 else lm_ref, ct % 2, ct, j * G, None)
            mc_ref[ct, pl.ds(j * G, G), :] = acc.astype(BF16)
    out_copy(0, 0, 0, BQ).wait()
    out_copy(1, 0, 0, BQ).wait()
    n = BQ + 16
    mo = jnp.dot(_cat(mc_ref, 0, n, (0, 1, 2, 3)), wmg_ref[...], preferred_element_type=F32)
    res = (x_ref[pl.ds((NS - 1) * BQ, n), :].astype(F32) + mo).astype(BF16)
    stage_ref[0] = res[:BQ]
    stage_ref[1, pl.ds(0, 16), :] = res[BQ:]
    c0 = out_copy(0, 0, (NS - 1) * BQ - 16, BQ)
    c1 = out_copy(1, 0, NS * BQ - 16, 16)
    c0.start()
    c1.start()
    c0.wait()
    c1.wait()


@jax.jit
def pallas_standalone__conformer_family_e_branchformer__speech_kernel(x, w_qkv, w_att_out, w_mlp_in, dw_csgu, w_mlp_out, dw_merge, w_merge):
    ws = (w_qkv, w_att_out, w_mlp_in, dw_csgu, w_mlp_out, dw_merge, w_merge)
    out = pl.pallas_call(
        _kernel,
        out_shape=jax.ShapeDtypeStruct((B * T, D), BF16),
        in_specs=[pl.BlockSpec(memory_space=pl.ANY)] * 8,
        out_specs=pl.BlockSpec(memory_space=pl.ANY),
        scratch_shapes=[pltpu.VMEM(w.shape, w.dtype) for w in ws] + [
            pltpu.VMEM((16 + B * T, D), BF16),
            pltpu.VMEM((2, B * T + 16, 128), BF16),
            pltpu.VMEM((3, TKP, 128), BF16),
            pltpu.VMEM((3, TKP, 128), BF16),
            pltpu.VMEM((BQ, TKP), F32),
            pltpu.VMEM((BQ, D), F32),
            pltpu.VMEM((BQ // 2, D), U32),
            pltpu.VMEM((2, BQ + 32, 128), F32),
            pltpu.VMEM((2, 16, 128), F32),
            pltpu.VMEM((2, BQ + 16, 128), F32),
            pltpu.VMEM((2, BQ + 32, 128), F32),
            pltpu.VMEM((2, 48, 128), F32),
            pltpu.VMEM((2, BQ + 32, 128), F32),
            pltpu.VMEM((2, 48, 128), F32),
            pltpu.VMEM((6, KT, 8, 128), F32),
            pltpu.VMEM((D, D), BF16),
            pltpu.VMEM((D, D), BF16),
            pltpu.VMEM((2, BQ, 128), BF16),
            pltpu.VMEM((4, BQ + 16, 128), BF16),
            pltpu.VMEM((2, BQ, D), BF16),
            pltpu.SemaphoreType.DMA((7,)),
            pltpu.SemaphoreType.DMA((NS,)),
            pltpu.SemaphoreType.DMA((2,)),
        ],
        compiler_params=pltpu.CompilerParams(vmem_limit_bytes=100 * 1024 * 1024),
    )(x.reshape(B * T, D), *ws)
    return out.reshape(B, T, D)
```

```python
import functools
import math

import jax
import jax.numpy as jnp
import jax.experimental.pallas as pl
import jax.experimental.pallas.tpu as pltpu

F32 = jnp.float32
BF16 = jnp.bfloat16
U32 = jnp.uint32

CFG = {}
B, T, D, KT = 2, 4000, 256, 31
HALO = KT // 2
BQ = 400
HQ = BQ // 2
NQ = T // BQ
NS = B * NQ
TKP = 4096
SUB = 512
NSUB = TKP // SUB
G = 16
NP = BQ // G
QROWS = 208
UROWS = BQ + 16
NZ = 32
C1 = CFG.get('C1', 6)
QD = CFG.get('QD', 1)
EARLY2 = CFG.get('EARLY2', 0)
SPLIT0 = CFG.get('SPLIT0', 0)
LATE1 = CFG.get('LATE1', 0)
PEEL_LAST = CFG.get('PEEL_LAST', 0)
ESPLIT = CFG.get('ESPLIT', (0, 13, 26))
EDMA = CFG.get('EDMA', 1)
XLROWS = 416
EPS = 1e-5
NEG = -1e30
LOG2E = math.log2(math.e)
GELU_C = math.sqrt(2.0 / math.pi)
QLINK = CFG.get("QLINK", 2)
PLINK = CFG.get("PLINK", 1)
GL_AT = CFG.get("GL_AT", 1)
HU_AT = CFG.get("HU_AT", 5)
HG_AT = CFG.get("HG_AT", 6)
MG_AT = CFG.get("MG_AT", 2)
LN_AT = CFG.get("LN_AT", 1)
QP_AT = CFG.get("QP_AT", 4)
HL = CFG.get("HL", 2)
RSPLIT = CFG.get("RSPLIT", 304)
LOC_LAST = CFG.get("LOC_LAST", 5)
LOC_FIRST = CFG.get("LOC_FIRST", 6)
UNROLL = CFG.get("UNROLL", 1)
CHAINX = CFG.get("CHAINX", 1)
OPQ = CFG.get("OPQ", 0)
UDB = CFG.get("UDB", 0)


def _pack(v):
    return pltpu.bitcast(v, U32)


def _unpack(v):
    return pltpu.bitcast(v, BF16)


def _mult(v, m):
    return v if isinstance(v, int) else pl.multiple_of(v, m)


def _cat(ref, r0, n, tiles):
    return _unpack(jnp.concatenate([ref[t, pl.ds(r0 // 2, n // 2), :] for t in tiles], axis=1))


def _catb(ref, r0, n, tiles=(0, 1)):
    return jnp.concatenate([ref[t, pl.ds(r0, n), :] for t in tiles], axis=1)


def _ln(v, eps):
    mu = jnp.mean(v, axis=-1, keepdims=True)
    c = v - mu
    var = jnp.mean(c * c, axis=-1, keepdims=True)
    return c * jnp.exp2(jnp.log(var + eps) * (-0.5 * LOG2E))


def _gelu2(h):
    z = h * ((h * h) * (GELU_C * 0.044715) + GELU_C)
    return h + h * jnp.tanh(z)


def _where(cond, a, b):
    if isinstance(cond, bool):
        return a if cond else jnp.full_like(a, b)
    return jnp.where(cond, a, b)


def _kernel(x_hbm, wqkv_hbm, wao_hbm, win_hbm, dwc_hbm, wout_hbm, dwm_hbm, wmg_hbm,
            out_hbm,
            wqkv_ref, wao_ref, win_ref, dwc_ref, wout_ref, dwm_ref, wmg_ref,
            x_ref, xl_ref, kv0_ref, kv1_ref, q0_ref, q1_ref, s_ref, acc_ref, pre_ref,
            gwin_ref, ghead_ref, u_ref, gm_ref, gm0_ref, lm_ref, lm0_ref, gm2_ref,
            cw_ref, wp_ref, ugc_ref, mcg_ref, mcl_ref, tmp_ref, o_ref, zero_ref,
            sem_in, sem_out):
    kv_refs = (kv0_ref, kv1_ref)
    q_refs = (q0_ref, q1_ref)
    W_A, W_VO, W_U, W_G, W_OUT, W_MG, W_ML = range(7)

    def mm(lhs, w):
        return jnp.dot(lhs, _unpack(wp_ref[w]), preferred_element_type=F32)

    def x_pair(c):
        if c == 0:
            return x_hbm.at[pl.ds(0, BQ), :], x_ref.at[0, pl.ds(16, BQ), :]
        return x_hbm.at[pl.ds(c * BQ - 16, BQ + 16), :], x_ref.at[c]

    def out_copy(c, r0=0, n=BQ, k=None):
        return pltpu.make_async_copy(o_ref.at[c, pl.ds(r0, n), :],
                                     out_hbm.at[pl.ds(_mult(c * BQ - 16 + r0, 16), n), :], sem_out.at[0])

    w_pairs = [(wqkv_hbm.at[:, pl.ds(0, 2 * D)], wqkv_ref.at[:, pl.ds(0, 2 * D)]),
               (dwc_hbm, dwc_ref), (dwm_hbm, dwm_ref), (win_hbm, win_ref),
               (wqkv_hbm.at[:, pl.ds(2 * D, D)], wqkv_ref.at[:, pl.ds(2 * D, D)]),
               (wao_hbm, wao_ref), (wout_hbm, wout_ref), (wmg_hbm, wmg_ref)]
    groups = [[x_pair(0), w_pairs[0]] + ([] if SPLIT0 else [x_pair(1)]),
              [x_pair(2), w_pairs[3], x_pair(3), w_pairs[1], w_pairs[2]] + [x_pair(c) for c in range(4, C1)],
              [x_pair(c) for c in range(C1, NQ + 1)] + w_pairs[4:],
              [x_pair(c) for c in range(NQ + 1, NS)],
              [x_pair(1)] if SPLIT0 else []]
    groups = [[pltpu.make_async_copy(src, dst, sem_in.at[k]) for src, dst in grp] for k, grp in enumerate(groups)]
    x_rest = groups[3]

    def ln_chunk(b, i, link=None):
        c = b * NQ + i
        h0 = _mult(i * HQ, 8)
        xv = x_ref[c, pl.ds(16, BQ), :]
        if link is not None:
            xv = link(xv)
        xa = _ln(xv.astype(F32), EPS)
        for ct in range(2):
            xt = xa[:, ct * 128:(ct + 1) * 128].astype(BF16)
            xl_ref[c, ct, pl.ds(BQ - 16, 16), :] = xt[:16]
            xl_ref[c + 1, ct, pl.ds(0, BQ - 16), :] = xt[16:]
        lo, hi = [jnp.concatenate([_pack(xl_ref[c, ct, pl.ds(BQ - 16, 16), :]),
                                   _pack(xl_ref[c + 1, ct, pl.ds(0, BQ - 16), :])], axis=0) for ct in range(2)]
        col = jax.lax.broadcasted_iota(jnp.int32, (HQ, 128), 1)
        kv = kv_refs[b]
        kv[0, pl.ds(h0, HQ), :] = lo
        kv[1, pl.ds(h0, HQ), :] = hi
        kv[2, pl.ds(h0, HQ), :] = jnp.where(col == 127, jnp.uint32(0x3F803F80), hi)
        return _unpack(jnp.concatenate([lo, hi], axis=1))

    def repack(v, slot=0):
        n = v.shape[0]
        for ct in range(2):
            tmp_ref[2 * slot + ct, pl.ds(0, n), :] = v[:, ct * 128:(ct + 1) * 128].astype(BF16)
        return _pack(_catb(tmp_ref, 0, n, (2 * slot, 2 * slot + 1)))

    def q_proj(b, i, xa=None):
        if xa is None:
            xa = _cat(kv_refs[b], i * BQ, BQ, (0, 1))
        q_refs[b][i, pl.ds(0, HQ), :] = repack(mm(xa, W_A), i % 2 if isinstance(i, int) else 0)

    def local_lhs(n):
        v = _catb(xl_ref.at[n + 1], 0, BQ)
        if isinstance(n, int) and n == 0:
            v = jnp.concatenate([_catb(xl_ref.at[0], BQ - 16, 16), v], axis=0)
        return v

    def local_u(n):
        return _gelu2(mm(local_lhs(n), W_U))

    def local_g(n):
        return _ln(_gelu2(mm(local_lhs(n), W_G)), 4.0 * EPS)

    def taps_sum(acc, src_ref, st, wt, w0, n, p0, link, zw):
        for k in range(n):
            wk_ = cw_ref[wt, zw + (w0 + k)]
            wk_ = jnp.concatenate([wk_] * (G // 8), axis=0)
            t = src_ref[st, pl.ds(p0 + k, G), :] * wk_
            if acc is None:
                acc = t if link is None else jnp.where(link[0], link[1], t)
            else:
                acc = acc + t
        return acc

    def conv_pair(src_ref, st, wt, c, mask, prev, zw=0, scale=None):
        p = taps_sum(None, src_ref, st, wt, KT, G, c + 1, None if prev is None else (mask, prev), zw)
        y0 = taps_sum(p, src_ref, 2 + st, wt, 0, G, c - HALO, None, zw)
        if scale is not None:
            y0 = y0 * scale[:G]
        p1 = p if mask is None else jnp.where(mask, y0, p)
        y1 = taps_sum(p1, src_ref, 2 + st, wt, KT + G, KT - G, c + 1, None, zw)
        if scale is not None:
            y1 = y1 * scale[G:]
        return y0, y1

    def normalized(acc):
        l = acc[:, D - 1:D]
        r = pl.reciprocal(l, approx=True)
        r = r * (2.0 - l * r)
        return (acc * r).astype(BF16)

    def push_block(win, win0, val, joined):
        for ct in range(2):
            new = val[:, ct * 128:(ct + 1) * 128]
            win0[ct, pl.ds(0, 32), :] = win[ct, pl.ds(BQ - 16, 32), :]
            tail = _where(joined, win[ct, pl.ds(BQ, 16), :], 0.0)
            win[ct, pl.ds(0, 16), :] = tail
            win[ct, pl.ds(16, BQ), :] = new
            win[2 + ct, pl.ds(0, BQ), :] = jnp.concatenate([tail, new[:BQ - 16]], axis=0) - new
            win0[ct, pl.ds(32, 16), :] = _where(joined, new[:16], 0.0)

    def startup0():
        for c in groups[0] + groups[4]:
            c.start()

        def clear(k, carry):
            zero_ref[k] = 0
            return carry
        jax.lax.fori_loop(0, NZ, clear, 0)
        x_ref[0, pl.ds(0, 16), :] = jnp.zeros((16, D), BF16)
        for ct in range(2):
            gwin_ref[ct, pl.ds(0, 16), :] = jnp.zeros((16, 128), F32)
            for r in (gm_ref, lm_ref):
                r[ct, pl.ds(BQ - 16, 48), :] = jnp.zeros((48, 128), F32)
            gm2_ref[ct, pl.ds(BQ + 32, 16), :] = jnp.zeros((16, 128), F32)
            xl_ref[NS, ct, pl.ds(BQ - 16, 16), :] = jnp.zeros((16, 128), BF16)
        for kv in kv_refs:
            for ct in range(3):
                kv[ct, pl.ds(T // 2, (TKP - T) // 2), :] = jnp.zeros(((TKP - T) // 2, 128), U32)
        if not LATE1:
            for c in groups[1]:
                c.start()
        for c in groups[0]:
            c.wait()
        if LATE1:
            for c in groups[1]:
                c.start()
        for c in groups[2][:EARLY2]:
            c.start()
        a = jax.lax.dot_general(wqkv_ref[:, 0:D], wqkv_ref[:, D:2 * D], (((1,), (1,)), ((), ())),
                                preferred_element_type=F32)
        wp_ref[W_A] = repack(a * (D ** -0.5 * LOG2E), 1)
        if SPLIT0:
            ln_chunk(0, 0)
            for c in groups[4]:
                c.wait()
            q_proj(0, 0)
        else:
            q_proj(0, 0, ln_chunk(0, 0))
        ln_chunk(0, 1)

    def startup1():
        for c in groups[1]:
            c.wait()
        for c in groups[2][EARLY2:]:
            c.start()
        q_proj(0, 1)
        wp_ref[W_U] = _pack(win_ref[:, 0:D])
        wp_ref[W_G] = _pack(win_ref[:, D:2 * D])
        u0 = local_u(0)
        g0 = local_g(0)
        for ct in range(2):
            gt = g0[:, ct * 128:(ct + 1) * 128]
            u_ref[ct, pl.ds(0, UROWS), :] = u0[:, ct * 128:(ct + 1) * 128]
            gwin_ref[ct, pl.ds(16, BQ + 16), :] = gt
            gwin_ref[2 + ct, pl.ds(0, BQ), :] = (
                jnp.concatenate([jnp.zeros((16, 128), F32), gt[:BQ - 16]], axis=0) - gt[:BQ])
            ghead_ref[ct] = gt[BQ:]
        dwm = dwm_ref[...].astype(F32)
        dwc = dwc_ref[...].astype(F32) * 0.5
        for wt in range(6):
            src = dwm if wt < 4 else dwc
            taps = [jnp.broadcast_to(src[k:k + 1, (wt % 4) * 128:(wt % 4 + 1) * 128], (8, 128)) for k in range(KT)]
            if wt < 4:
                taps[HALO] = taps[HALO] + 1.0
            for k in range(KT):
                cw_ref[wt, k] = taps[k]
            for k in range(G):
                cw_ref[wt, KT + k] = taps[k] + taps[G + k] if G + k < KT else taps[k]
            for k in range(KT - G):
                cw_ref[wt, KT + G + k] = -taps[G + k]
        for c in range(2, C1):
            ln_chunk(0, c)
        for c in range(2, C1 - QD):
            q_proj(0, c)

    def startup3():
        for c in groups[2]:
            c.wait()
        for c in x_rest:
            c.start()
        for c in range(C1 - QD, C1):
            q_proj(0, c)
        wvo = jnp.dot(wqkv_ref[:, 2 * D:3 * D], wao_ref[...], preferred_element_type=F32)
        wp_ref[W_VO] = repack(wvo - wvo[D - 1:D, :], 2)
        wp_ref[W_OUT] = _pack(wout_ref[...])
        wp_ref[W_MG] = _pack(wmg_ref[0:D, :])
        wp_ref[W_ML] = _pack(wmg_ref[D:2 * D, :])
        for c in range(C1, NQ):
            ln_chunk(0, c)

    def startup4():
        for c in range(C1, NQ):
            q_proj(0, c)

    def step(b, i, state):
        static = isinstance(i, int)
        s = b * NQ + i
        first = static and s == 0
        last = static and s == NS - 1
        kv = kv_refs[b]
        slot = s % 2
        ucur = _mult(slot * UROWS, 32) if UDB else 0
        unxt = _mult((1 - slot) * UROWS, 32) if UDB else 0
        hooks = {1: startup1, 3: startup3, 4: startup4} if first else {}
        if first:
            startup0()

        zero = zero_ref[0]
        zoff = pl.multiple_of(zero, 32)
        zq = zoff if OPQ else 0
        negs = -(jax.lax.broadcasted_iota(jnp.int32, (8, 128), 0) + zero) - 1

        def never(rows):
            return jnp.concatenate([negs] * (rows // 8), axis=0) >= 0

        def link_packed(v, dep):
            nv = never(HQ)
            du = _pack(dep)
            return jnp.concatenate([jnp.where(nv, du[:HQ], v[:, :128]),
                                    jnp.where(nv, du[HQ:], v[:, 128:])], axis=1)

        never_g = never(G)
        snext = s + 1 if (static or b == 0 or PEEL_LAST) else jnp.minimum(s + 1, NS - 1)

        def chain(src_ref, st, wt, c, scale=None):
            zw = zero_ref[state["n"] % NZ]
            link = None if state["prev"] is None else (never_g, state["prev"])
            acc = taps_sum(None, src_ref, st, wt, 0, KT, zoff + (c - HALO), link, zw)
            if scale is not None:
                acc = acc * scale
            state["prev"] = acc
            state["n"] += 1
            return acc

        def chain2(src_ref, st, wt, c, scale=None):
            zw = zero_ref[state["n"] % NZ]
            y0, y1 = conv_pair(src_ref, st, wt, zoff + c, never_g, state["prev"], zw, scale)
            state["prev"] = y1
            state["n"] += 1
            return jnp.concatenate([y0, y1], axis=0)

        def m_pieces(cts, n=NP):
            for ct in cts:
                win, win0, dst = (gm_ref, gm0_ref, mcg_ref) if ct < 2 else (lm_ref, lm0_ref, mcl_ref)
                dst[ct % 2, pl.ds(0, G), :] = chain(win0, ct % 2, ct, 16).astype(BF16)
                for j in range(1, NP, 2):
                    dst[ct % 2, pl.ds(j * G, 2 * G), :] = chain2(win, ct % 2, ct, j * G).astype(BF16)
                if n > NP:
                    dst[ct % 2, pl.ds(NP * G, G), :] = chain(win, ct % 2, ct, NP * G).astype(BF16)

        def g_pieces():
            for ct in range(2):
                for j in range(0, NP, 2):
                    n = G if j == NP - 1 else 2 * G
                    acc = (chain if j == NP - 1 else chain2)(gwin_ref, ct, 4 + ct, 16 + j * G,
                                                             u_ref[ct, pl.ds(ucur + j * G, n), :])
                    ugc_ref[ct, pl.ds(j * G, n), :] = acc.astype(BF16)

        def merge_glob():
            mo = mm(_catb(mcg_ref, 0, BQ), W_MG)
            o_ref[s - 1, pl.ds(0, BQ), :] = (pre_ref[pl.ds(zq, BQ), :] + mo).astype(BF16)

        nl = BQ + 16 if last else BQ

        def local_out():
            push_block(lm_ref, lm0_ref, mm(_catb(ugc_ref, 0, BQ), W_OUT), i != 0)
            m_pieces((2, 3), nl // G)

        if not first:
            g_pieces()

        mms = []
        pend = {}
        loc_at = LOC_FIRST if first else LOC_LAST if last else NSUB - 1
        for sb in range(NSUB):
            if sb in hooks:
                hooks[sb]()
                if sb == 3:
                    g_pieces()
            qs = q_refs[b][i, pl.ds(0, HQ), :]
            if sb >= QLINK:
                qs = link_packed(qs, mms[sb - QLINK])
            for dep in pend.pop(sb, []):
                qs = link_packed(qs, dep)
            kc = _cat(kv, sb * SUB, SUB, (0, 1))
            sc = jax.lax.dot_general(_unpack(qs), kc, (((1,), (1,)), ((), ())), preferred_element_type=F32)
            if sb == NSUB - 1:
                nvalid = T - (TKP - 128)
                col = jax.lax.broadcasted_iota(jnp.int32, (BQ, 128), 1)
                tail = jnp.where(col < nvalid, sc[:, SUB - 128:], NEG)
                sc = jnp.concatenate([sc[:, :SUB - 128], tail], axis=1)
            s_ref[:, sb * SUB:(sb + 1) * SUB] = sc
            mx = sc[:, 0:128] if sb == 0 else jnp.maximum(mms[-1], sc[:, 0:128])
            for t in range(1, SUB // 128):
                mx = jnp.maximum(mx, sc[:, t * 128:(t + 1) * 128])
            mms.append(mx)
            if sb == GL_AT and not first:
                push_block(gm_ref, gm0_ref, mm(normalized(acc_ref[pl.ds(zq, BQ), :]), W_VO), i != 1)
                m_pieces((0, 1))
                if last:
                    for ct in range(2):
                        gm2_ref[ct, pl.ds(0, 32), :] = gm_ref[ct, pl.ds(BQ - 16, 32), :]
            if sb == loc_at and sb < NSUB - 1:
                local_out()
            if sb == HU_AT and not last:
                u = local_u(snext)
                pend.setdefault(sb + HL, []).extend([u[:, :128], u[:, 128:]])
                for ct in range(2):
                    u_ref[ct, pl.ds(unxt, 16), :] = u_ref[ct, pl.ds(ucur + BQ, 16), :]
                    u_ref[ct, pl.ds(unxt + 16, BQ), :] = u[:, ct * 128:(ct + 1) * 128]
            if sb == HG_AT and not last:
                g = local_g(snext)
                pend.setdefault(sb + HL, []).extend([g[:, :128], g[:, 128:]])
                for ct in range(2):
                    gt = g[:, ct * 128:(ct + 1) * 128]
                    full = jnp.concatenate([_where(i != NQ - 1, gwin_ref[ct, pl.ds(BQ, 16), :], 0.0),
                                            ghead_ref[ct], gt[:BQ - 16]], axis=0)
                    gwin_ref[ct, pl.ds(0, BQ + 16), :] = full
                    gwin_ref[2 + ct, pl.ds(0, BQ), :] = full[:BQ] - full[16:]
                    gwin_ref[ct, pl.ds(BQ + 16, 16), :] = _where(i != NQ - 2, gt[BQ - 16:], 0.0)
                    ghead_ref[ct] = gt[BQ - 16:]
        mx = jnp.broadcast_to(jnp.max(mms[-1], axis=1, keepdims=True), (BQ, 128))
        if loc_at == NSUB - 1:
            local_out()

        def merge_loc():
            mo = mm(_catb(mcl_ref, 0, nl), W_ML)
            pre_ref[pl.ds(0, nl), :] = x_ref[s, pl.ds(0, nl), :].astype(F32) + mo

        def pv_acc(r0, r1, sb, dep):
            mxs = mx[r0:r1]
            for d in dep:
                mxs = jnp.where(never(r1 - r0), d, mxs)
            p = jnp.exp2(s_ref[pl.ds(r0, r1 - r0), sb * SUB:(sb + 1) * SUB]
                         - jnp.concatenate([mxs] * (SUB // 128), axis=1))
            pv = jnp.dot(p.astype(BF16), _cat(kv, sb * SUB, SUB, (0, 2)), preferred_element_type=F32)
            if sb == 0:
                acc_ref[pl.ds(r0, r1 - r0), :] = pv
            else:
                acc_ref[pl.ds(r0, r1 - r0), :] += pv
            return pv[:, :128]

        r1 = RSPLIT if last else BQ
        pvs = []
        xa_next = None
        for sb in range(NSUB):
            dep = ([pvs[sb - PLINK]] if sb >= PLINK else []) + pend.pop(NSUB + sb, [])
            pvs.append(pv_acc(0, r1, sb, dep))
            if sb == MG_AT and not first:
                merge_glob()
            if sb == LN_AT and b + 1 < B:
                lnk = pvs[sb]
                xa_next = ln_chunk(b + 1, i, lambda xv: _unpack(link_packed(_pack(xv), lnk)))
            if sb == QP_AT and b + 1 < B:
                q_proj(b + 1, i, xa_next)
        merge_loc()
        if not last:
            return

        j1, j2 = (r1 - 14 + G - 1) // G // 2 * 2, NP + 1

        def glob_rows(ra, rb, final):
            glob = mm(normalized(acc_ref[pl.ds(ra, rb - ra), :]), W_VO)
            for ct in range(2):
                gt = glob[:, ct * 128:(ct + 1) * 128]
                d0 = 0 if ra == 0 else ra + 16
                full = jnp.concatenate([gm2_ref[ct, pl.ds(d0, 32 + ra - d0), :], gt]
                                       + ([jnp.zeros((16, 128), F32)] if final else []), axis=0)
                gm2_ref[ct, pl.ds(32 + ra, rb - ra), :] = gt
                gm2_ref[2 + ct, pl.ds(d0, full.shape[0] - 16), :] = full[:-16] - full[16:]

        def merge2(ja, jb, chained):
            cols = []
            for ct in range(2):
                state["prev"] = None
                rows = []
                for j in range(ja, jb, 2):
                    if chained:
                        rows.append(chain2(gm2_ref, ct, ct, 16 + j * G))
                    else:
                        rows.extend(conv_pair(gm2_ref, ct, ct, zoff + 16 + j * G, None, None))
                cols.append(jnp.concatenate(rows, axis=0))
            lhs = jnp.concatenate(cols, axis=1).astype(BF16)

            def finish():
                oa, n = ja * G, (jb - ja) * G
                o_ref[s, pl.ds(oa, n), :] = (pre_ref[pl.ds(oa, n), :] + mm(lhs, W_MG)).astype(BF16)
            return finish

        glob_rows(0, r1, False)
        finish = merge2(0, j1, True)
        hist = []
        for sb in range(NSUB):
            hist.append(pv_acc(r1, BQ, sb, [hist[-2]] if sb >= 2 else []))
        finish()
        glob_rows(r1, BQ, True)
        copies = [out_copy(s - 1), out_copy(s, 0, j1 * G), out_copy(s, j1 * G, (j2 - j1) * G, NS)]
        copies[0].start()
        copies[1].start()
        merge2(j1, j2, False)()
        copies[2].start()
        state["copies"] = copies

    def block(b, it, carry):
        i = it + (1 - b)
        step(b, i, {"prev": None, "n": 0})
        if b == 0:
            @pl.when(i == 1)
            def _():
                out_copy(0, 16, BQ - 16).start()

            @pl.when(i > 1)
            def _():
                out_copy(i - 1).start()
        else:
            out_copy(NQ + i - 1).start()
        return carry

    step(0, 0, {"prev": None, "n": 0})
    for c in x_rest:
        c.wait()
    jax.lax.fori_loop(0, NQ - 1, functools.partial(block, 0), 0)
    jax.lax.fori_loop(0, NQ - 1 if PEEL_LAST else NQ, functools.partial(block, 1), 0)
    if PEEL_LAST:
        fin = {"prev": None, "n": 0}
        step(B - 1, NQ - 1, fin)
        copies = fin["copies"]
    else:
        s = NS - 1
        zoff = pl.multiple_of(zero_ref[0], 32)
        push_block(gm_ref, gm0_ref, mm(normalized(acc_ref[...]), W_VO), True)
        tail = jnp.concatenate([taps_sum(None, lm_ref, ct, 2 + ct, 0, KT, BQ - HALO, None, 0) for ct in range(2)], axis=1)
        pre_ref[pl.ds(BQ, 16), :] = x_ref[s, pl.ds(BQ, 16), :].astype(F32) + mm(tail.astype(BF16), W_ML)
        copies = []
        for e in range(len(ESPLIT) - 1):
            ja, jb = ESPLIT[e], ESPLIT[e + 1]
            cols = []
            for ct in range(2):
                rows = []
                j = ja
                while j < jb:
                    if j == 0:
                        rows.append(taps_sum(None, gm0_ref, ct, ct, 0, KT, zoff + (16 - HALO), None, 0))
                        j += 1
                    elif j == NP:
                        rows.append(taps_sum(None, gm_ref, ct, ct, 0, KT, zoff + (j * G - HALO), None, 0))
                        j += 1
                    else:
                        rows.extend(conv_pair(gm_ref, ct, ct, zoff + j * G, None, None))
                        j += 2
                cols.append(jnp.concatenate(rows, axis=0))
            lhs = jnp.concatenate(cols, axis=1).astype(BF16)
            oa, n = ja * G, (jb - ja) * G
            o_ref[s, pl.ds(oa, n), :] = (pre_ref[pl.ds(oa, n), :] + mm(lhs, W_MG)).astype(BF16)
            if EDMA or e == len(ESPLIT) - 2:
                r0 = oa if EDMA else 0
                copies.append(out_copy(s, r0, oa + n - r0, s + e if EDMA else s))
                copies[-1].start()
    pltpu.make_async_copy(out_hbm, out_hbm, sem_out.at[0]).wait()


@jax.jit
def pallas_standalone__conformer_family_e_branchformer__speech_kernel(x, w_qkv, w_att_out, w_mlp_in, dw_csgu, w_mlp_out, dw_merge, w_merge):
    ws = (w_qkv, w_att_out, w_mlp_in, dw_csgu, w_mlp_out, dw_merge, w_merge)
    out = pl.pallas_call(
        _kernel,
        out_shape=jax.ShapeDtypeStruct((B * T, D), BF16),
        in_specs=[pl.BlockSpec(memory_space=pl.ANY)] * 8,
        out_specs=pl.BlockSpec(memory_space=pl.ANY),
        scratch_shapes=[pltpu.VMEM(w.shape, w.dtype) for w in ws] + [
            pltpu.VMEM((NS, BQ + 16, D), BF16),
            pltpu.VMEM((NS + 1, 2, XLROWS, 128), BF16),
            pltpu.VMEM((3, TKP // 2, 128), U32),
            pltpu.VMEM((3, TKP // 2, 128), U32),
            pltpu.VMEM((NQ, QROWS, D), U32),
            pltpu.VMEM((NQ, QROWS, D), U32),
            pltpu.VMEM((BQ, TKP), F32),
            pltpu.VMEM((BQ, D), F32),
            pltpu.VMEM((BQ + 16, D), F32),
            pltpu.VMEM((4, BQ + 32, 128), F32),
            pltpu.VMEM((2, 16, 128), F32),
            pltpu.VMEM((2, 2 * UROWS, 128), F32),
            pltpu.VMEM((4, BQ + 32, 128), F32),
            pltpu.VMEM((2, 48, 128), F32),
            pltpu.VMEM((4, BQ + 32, 128), F32),
            pltpu.VMEM((2, 48, 128), F32),
            pltpu.VMEM((4, BQ + 48, 128), F32),
            pltpu.VMEM((6, 2 * KT, 8, 128), F32),
            pltpu.VMEM((7, D // 2, D), U32),
            pltpu.VMEM((2, BQ, 128), BF16),
            pltpu.VMEM((2, BQ, 128), BF16),
            pltpu.VMEM((2, BQ + 16, 128), BF16),
            pltpu.VMEM((6, BQ, 128), BF16),
            pltpu.VMEM((NS, BQ + 16, D), BF16),
            pltpu.SMEM((NZ,), jnp.int32),
            pltpu.SemaphoreType.DMA((5,)),
            pltpu.SemaphoreType.DMA((1,)),
        ],
        compiler_params=pltpu.CompilerParams(vmem_limit_bytes=100 * 1024 * 1024),
    )(x.reshape(B * T, D), *ws)
    return out.reshape(B, T, D)
```

```python
import functools
import math

import jax
import jax.numpy as jnp
import jax.experimental.pallas as pl
import jax.experimental.pallas.tpu as pltpu

F32 = jnp.float32
BF16 = jnp.bfloat16
U32 = jnp.uint32

B, T, D, KT = 2, 4000, 256, 31
HALO = KT // 2
BQ = 400
HQ = BQ // 2
NQ = T // BQ
NS = B * NQ
TKP = 4096
NT = T % 128
SUB = 512
NSUB = TKP // SUB
G = 16
NP = BQ // G
BP = BQ + 16
NZ = 32
EPS = 1e-5
NEG = -1e30
LOG2E = math.log2(math.e)
GELU_C = math.sqrt(2.0 / math.pi)
NT_DIMS = (((1,), (1,)), ((), ()))
QLINK = 2
LN_AT = 1
QP_AT = 4
C1 = 6
G0_AT = 5
TSCHED = {1: (0,), 3: (1, 2), 4: (3, 4), 5: (5,), 6: (6,), 7: (7,)}
RSPLIT = 272
ESPLIT = (0, 16, 26)


def _pack(v):
    return pltpu.bitcast(v, U32)


def _unpack(v):
    return pltpu.bitcast(v, BF16)


def _nt(a, b):
    return jax.lax.dot_general(a, b, NT_DIMS, preferred_element_type=F32)


def _cat(ref, r0, n):
    return _unpack(jnp.concatenate([ref[t, pl.ds(r0 // 2, n // 2), :] for t in range(2)], axis=1))


def _catb(ref, r0, n, tiles=(0, 1)):
    return jnp.concatenate([ref[t, pl.ds(r0, n), :] for t in tiles], axis=1)


def _ln(v, eps):
    mu = jnp.mean(v, axis=-1, keepdims=True)
    c = v - mu
    var = jnp.mean(c * c, axis=-1, keepdims=True)
    return c * jnp.exp2(jnp.log(var + eps) * (-0.5 * LOG2E))


def _gelu2(h):
    z = h * ((h * h) * (GELU_C * 0.044715) + GELU_C)
    return h + h * jnp.tanh(z)


def _where(cond, a, b):
    if isinstance(cond, bool):
        return a if cond else jnp.full_like(a, b)
    return jnp.where(cond, a, b)


def _kernel(x_hbm, wqkv_hbm, wao_hbm, win_hbm, dwc_hbm, wout_hbm, dwm_hbm, wmg_hbm,
            out_hbm,
            wqkv_ref, wao_ref, win_ref, dwc_ref, wout_ref, dwm_ref, wmg_ref,
            x_ref, xl_ref, k_ref, v0_ref, v1_ref, q_ref, s_ref, mx_ref, acc_ref, pre_ref,
            gwin_ref, ghead_ref, u_ref, gm_ref, gm0_ref, lm_ref, lm0_ref, gm2_ref,
            xt_ref, zt_ref, str_ref, st_ref, cw_ref, wp_ref, ugc_ref, mc_ref, tmp_ref, o_ref, zero_ref,
            sem_in, sem_out):
    v_refs = (v0_ref, v1_ref)
    W_A, W_VO, W_U, W_G, W_OUT, W_MG, W_ML = range(7)

    def mm(lhs, *ws):
        w = jnp.concatenate([wp_ref[k] for k in ws], axis=0)
        return jnp.dot(lhs, _unpack(w), preferred_element_type=F32)

    def x_pair(c):
        if c == 0:
            return x_hbm.at[pl.ds(0, BQ), :], x_ref.at[0, pl.ds(16, BQ), :]
        return x_hbm.at[pl.ds(c * BQ - 16, BP), :], x_ref.at[c]

    def out_copy(c, r0=0, n=BQ):
        dst = c * BQ - 16 + r0
        if not isinstance(dst, int):
            dst = pl.multiple_of(dst, 16)
        return pltpu.make_async_copy(o_ref.at[c, pl.ds(r0, n), :], out_hbm.at[pl.ds(dst, n), :], sem_out.at[0])

    w_pairs = [(wqkv_hbm.at[:, pl.ds(0, 2 * D)], wqkv_ref.at[:, pl.ds(0, 2 * D)]),
               (dwc_hbm, dwc_ref), (dwm_hbm, dwm_ref), (win_hbm, win_ref),
               (wqkv_hbm.at[:, pl.ds(2 * D, D)], wqkv_ref.at[:, pl.ds(2 * D, D)]),
               (wao_hbm, wao_ref), (wout_hbm, wout_ref), (wmg_hbm, wmg_ref)]
    t_pairs = [(x_hbm.at[pl.ds((b + 1) * T - NT, NT), :], xt_ref.at[pl.ds(b * NT, NT), :]) for b in range(B)]
    groups = [[w_pairs[0], x_pair(0), x_pair(1)] + t_pairs,
              [x_pair(2), w_pairs[3]] + [x_pair(c) for c in range(3, C1)],
              [x_pair(c) for c in range(C1, NQ)] + w_pairs[4:],
              [x_pair(c) for c in range(NQ, NS)],
              [w_pairs[1], w_pairs[2]]]
    groups = [[pltpu.make_async_copy(src, dst, sem_in.at[k]) for src, dst in grp] for k, grp in enumerate(groups)]

    def start(k):
        for c in groups[k]:
            c.start()

    def wait(k):
        for c in groups[k]:
            c.wait()

    def ln_chunk(b, i, link=None):
        c = b * NQ + i
        h0 = i * HQ if isinstance(i, int) else pl.multiple_of(i * HQ, 8)
        xv = x_ref[c, pl.ds(16, BQ), :]
        if link is not None:
            xv = link(xv)
        xa = _ln(xv.astype(F32), EPS)
        for ct in range(2):
            xt = xa[:, ct * 128:(ct + 1) * 128].astype(BF16)
            xl_ref[c, ct, pl.ds(BQ - 16, 16), :] = xt[:16]
            xl_ref[c + 1, ct, pl.ds(0, BQ - 16), :] = xt[16:]
        lo, hi = [jnp.concatenate([_pack(xl_ref[c, ct, pl.ds(BQ - 16, 16), :]),
                                   _pack(xl_ref[c + 1, ct, pl.ds(0, BQ - 16), :])], axis=0) for ct in range(2)]
        col = jax.lax.broadcasted_iota(jnp.int32, (HQ, 128), 1)
        k_ref[b, 0, pl.ds(h0, HQ), :] = lo
        k_ref[b, 1, pl.ds(h0, HQ), :] = hi
        v_refs[b][0, pl.ds(h0, HQ), :] = lo
        v_refs[b][1, pl.ds(h0, HQ), :] = jnp.where(col == 127, jnp.uint32(0x3F803F80), hi)
        return _unpack(jnp.concatenate([lo, hi], axis=1))

    def repack(v, slot=0):
        n = v.shape[0]
        for ct in range(2):
            tmp_ref[2 * slot + ct, pl.ds(0, n), :] = v[:, ct * 128:(ct + 1) * 128].astype(BF16)
        return _pack(_catb(tmp_ref, 0, n, (2 * slot, 2 * slot + 1)))

    def q_proj(b, i, xa=None):
        if xa is None:
            xa = _cat(k_ref.at[b], i * BQ, BQ)
        q_ref[b * NQ + i, pl.ds(0, HQ), :] = repack(mm(xa, W_A), i % 2 if isinstance(i, int) else 0)

    def tail_scores(st):
        n = st.shape[1]
        return jnp.transpose(jnp.concatenate([st, jnp.full((128 - NT, n), NEG, F32)], axis=0))

    def local_lhs(n):
        v = _catb(xl_ref.at[n + 1], 0, BQ)
        if isinstance(n, int) and n == 0:
            v = jnp.concatenate([_catb(xl_ref.at[0], BQ - 16, 16), v], axis=0)
        return v

    def local_u(n):
        return _gelu2(mm(local_lhs(n), W_U))

    def local_g(n):
        return _ln(_gelu2(mm(local_lhs(n), W_G)), 4.0 * EPS)

    def taps_sum(acc, src_ref, st, wt, w0, n, p0, link, zw):
        for k in range(n):
            wk_ = cw_ref[wt, zw + (w0 + k)]
            wk_ = jnp.concatenate([wk_] * (G // 8), axis=0)
            t = src_ref[st, pl.ds(p0 + k, G), :] * wk_
            if acc is None:
                acc = t if link is None else jnp.where(link[0], link[1], t)
            else:
                acc = acc + t
        return acc

    def conv_pair(src_ref, st, wt, c, mask, prev, zw, scale=None):
        p = taps_sum(None, src_ref, st, wt, KT, G, c + 1, None if prev is None else (mask, prev), zw)
        y0 = taps_sum(p, src_ref, 2 + st, wt, 0, G, c - HALO, None, zw)
        if scale is not None:
            y0 = y0 * scale[:G]
        p1 = p if mask is None else jnp.where(mask, y0, p)
        y1 = taps_sum(p1, src_ref, 2 + st, wt, KT + G, KT - G, c + 1, None, zw)
        if scale is not None:
            y1 = y1 * scale[G:]
        return y0, y1

    def normalized(acc):
        l = acc[:, D - 1:D]
        r = pl.reciprocal(l, approx=True)
        r = r * (2.0 - l * r)
        return (acc * r).astype(BF16)

    def push_block(win, win0, val, joined):
        for ct in range(2):
            new = val[:, ct * 128:(ct + 1) * 128]
            win0[ct, pl.ds(0, 32), :] = win[ct, pl.ds(BQ - 16, 32), :]
            tail = _where(joined, win[ct, pl.ds(BQ, 16), :], 0.0)
            win[ct, pl.ds(0, 16), :] = tail
            win[ct, pl.ds(16, BQ), :] = new
            win[2 + ct, pl.ds(0, BQ), :] = jnp.concatenate([tail, new[:BQ - 16]], axis=0) - new
            win0[ct, pl.ds(32, 16), :] = _where(joined, new[:16], 0.0)

    def startup0():
        start(4)
        start(0)

        def clear(k, carry):
            zero_ref[k] = 0
            return carry
        jax.lax.fori_loop(0, NZ, clear, 0)
        x_ref[0, pl.ds(0, 16), :] = jnp.zeros((16, D), BF16)
        pad = jnp.zeros(((TKP - T) // 2, 128), U32)
        for ct in range(2):
            gwin_ref[ct, pl.ds(0, 16), :] = jnp.zeros((16, 128), F32)
            for r in (gm_ref, lm_ref):
                r[ct, pl.ds(BQ - 16, 48), :] = jnp.zeros((48, 128), F32)
            gm2_ref[ct, pl.ds(BQ + 32, 16), :] = jnp.zeros((16, 128), F32)
            xl_ref[NS, ct, pl.ds(BQ - 16, 16), :] = jnp.zeros((16, 128), BF16)
            for b in range(B):
                k_ref[b, ct, pl.ds(T // 2, (TKP - T) // 2), :] = pad
                v_refs[b][ct, pl.ds(T // 2, (TKP - T) // 2), :] = pad
        wait(4)
        dwm = dwm_ref[...].astype(F32)
        dwc = dwc_ref[...].astype(F32) * 0.5
        for wt in range(6):
            src = dwm if wt < 4 else dwc
            taps = [jnp.broadcast_to(src[k:k + 1, (wt % 4) * 128:(wt % 4 + 1) * 128], (8, 128)) for k in range(KT)]
            if wt < 4:
                taps[HALO] = taps[HALO] + 1.0
            for k in range(KT):
                cw_ref[wt, k] = taps[k]
            for k in range(G):
                cw_ref[wt, KT + k] = taps[k] + taps[G + k] if G + k < KT else taps[k]
            for k in range(KT - G):
                cw_ref[wt, KT + G + k] = -taps[G + k]
        start(1)
        wait(0)
        a = _nt(wqkv_ref[:, 0:D], wqkv_ref[:, D:2 * D])
        wp_ref[W_A] = repack(a * (D ** -0.5 * LOG2E), 1)
        q_proj(0, 0, ln_chunk(0, 0))
        kt = _ln(xt_ref[...].astype(F32), EPS).astype(BF16)
        zt_ref[...] = repack(_nt(kt, _unpack(wp_ref[W_A])), 2)
        ln_chunk(0, 1)

    def startup1():
        wait(1)
        start(2)
        q_proj(0, 1)
        wp_ref[W_U] = _pack(win_ref[:, 0:D])
        wp_ref[W_G] = _pack(win_ref[:, D:2 * D])
        u0 = local_u(0)
        g0 = local_g(0)
        for ct in range(2):
            gt = g0[:, ct * 128:(ct + 1) * 128]
            u_ref[ct] = u0[:, ct * 128:(ct + 1) * 128]
            gwin_ref[ct, pl.ds(16, BP), :] = gt
            gwin_ref[2 + ct, pl.ds(0, BQ), :] = (
                jnp.concatenate([jnp.zeros((16, 128), F32), gt[:BQ - 16]], axis=0) - gt[:BQ])
            ghead_ref[ct] = gt[BQ:]
        for c in range(2, C1):
            ln_chunk(0, c)
        for c in range(2, C1 - 1):
            q_proj(0, c)

    def startup3():
        wait(2)
        start(3)
        q_proj(0, C1 - 1)
        wp_ref[W_OUT] = _pack(wout_ref[...])
        wp_ref[W_MG] = _pack(wmg_ref[0:D, :])
        wp_ref[W_ML] = _pack(wmg_ref[D:2 * D, :])
        for c in range(C1, NQ):
            ln_chunk(0, c)

    def startup4():
        for c in range(C1, NQ - 1):
            q_proj(0, c)

    def startup_end():
        q_proj(0, NQ - 1)
        wvo = jnp.dot(wqkv_ref[:, 2 * D:3 * D], wao_ref[...], preferred_element_type=F32)
        wp_ref[W_VO] = repack(wvo - wvo[D - 1:D, :], 2)

    def block(b, i, carry=None):
        static = isinstance(i, int)
        s = b * NQ + i
        first = static and s < 0
        last = static and s == NS - 1
        if first:
            startup0()

        zero = zero_ref[0]
        zoff = pl.multiple_of(zero, 32)
        negs = -(jax.lax.broadcasted_iota(jnp.int32, (8, 128), 0) + zero) - 1
        state = {"prev": None, "n": 0}

        def never(rows):
            return jnp.concatenate([negs] * (rows // 8), axis=0) >= 0

        def link_packed(v, dep):
            nv = never(HQ)
            du = _pack(dep)
            return jnp.concatenate([jnp.where(nv, du[:HQ], v[:, :128]),
                                    jnp.where(nv, du[HQ:], v[:, 128:])], axis=1)

        never_g = never(G)

        def next_zero():
            state["n"] += 1
            return zero_ref[(state["n"] - 1) % NZ]

        def chain(src_ref, st, wt, c, scale=None):
            link = None if state["prev"] is None else (never_g, state["prev"])
            acc = taps_sum(None, src_ref, st, wt, 0, KT, zoff + (c - HALO), link, next_zero())
            if scale is not None:
                acc = acc * scale
            state["prev"] = acc
            return acc

        def chain2(src_ref, st, wt, c, scale=None):
            y0, y1 = conv_pair(src_ref, st, wt, zoff + c, never_g, state["prev"], next_zero(), scale)
            state["prev"] = y1
            return jnp.concatenate([y0, y1], axis=0)

        def merge_conv(cts, n=NP):
            for ct in cts:
                win, win0 = (gm_ref, gm0_ref) if ct < 2 else (lm_ref, lm0_ref)
                mc_ref[ct, pl.ds(0, G), :] = chain(win0, ct % 2, ct, 16).astype(BF16)
                for j in range(1, NP, 2):
                    mc_ref[ct, pl.ds(j * G, 2 * G), :] = chain2(win, ct % 2, ct, j * G).astype(BF16)
                if n > NP:
                    mc_ref[ct, pl.ds(NP * G, G), :] = chain(win, ct % 2, ct, NP * G).astype(BF16)

        def gate_conv():
            for ct in range(2):
                for j in range(0, NP, 2):
                    n = G if j == NP - 1 else 2 * G
                    acc = (chain if j == NP - 1 else chain2)(gwin_ref, ct, 4 + ct, 16 + j * G,
                                                             u_ref[ct, pl.ds(j * G, n), :])
                    ugc_ref[ct, pl.ds(j * G, n), :] = acc.astype(BF16)

        def pv_acc(r0, r1, sb, dep):
            mxs = mx_ref[pl.ds(r0, r1 - r0), :]
            for d in dep:
                mxs = jnp.where(never(r1 - r0), d, mxs)
            p = jnp.exp2(s_ref[pl.ds(r0, r1 - r0), sb * SUB:(sb + 1) * SUB]
                         - jnp.concatenate([mxs] * (SUB // 128), axis=1))
            pv = jnp.dot(p.astype(BF16), _cat(v_refs[b], sb * SUB, SUB), preferred_element_type=F32)
            if sb == 0:
                acc_ref[pl.ds(r0, r1 - r0), :] = pv
            else:
                acc_ref[pl.ds(r0, r1 - r0), :] += pv
            return pv[:, :128]

        pvs = []
        if not first:
            r1 = RSPLIT if last else BQ
            dep = []
            if not last:
                u = local_u(s + 1)
                for ct in range(2):
                    u_ref[ct, pl.ds(0, 16), :] = u_ref[ct, pl.ds(BQ, 16), :]
                    u_ref[ct, pl.ds(16, BQ), :] = u[:, ct * 128:(ct + 1) * 128]
                g = local_g(s + 1)
                for ct in range(2):
                    gt = g[:, ct * 128:(ct + 1) * 128]
                    full = jnp.concatenate([_where(i != NQ - 1, gwin_ref[ct, pl.ds(BQ, 16), :], 0.0),
                                            ghead_ref[ct], gt[:BQ - 16]], axis=0)
                    gwin_ref[ct, pl.ds(0, BP), :] = full
                    gwin_ref[2 + ct, pl.ds(0, BQ), :] = full[:BQ] - full[16:]
                    gwin_ref[ct, pl.ds(BP, 16), :] = _where(i != NQ - 2, gt[BQ - 16:], 0.0)
                    ghead_ref[ct] = gt[BQ - 16:]
                dep = [u[:, :128], u[:, 128:], g[:, :128], g[:, 128:]]
            push_block(lm_ref, lm0_ref, mm(_catb(ugc_ref, 0, BQ), W_OUT), i != 0)
            merge_conv((2, 3), NP + 1 if last else NP)
            if not last:
                gate_conv()
            xa_next = None
            for sb in range(NSUB):
                pvs.append(pv_acc(0, r1, sb, dep))
                dep = [pvs[sb]]
                if sb == LN_AT and b + 1 < B:
                    lnk = pvs[sb]
                    xa_next = ln_chunk(b + 1, i, lambda xv: _unpack(link_packed(_pack(xv), lnk)))
                if sb == QP_AT and b + 1 < B:
                    q_proj(b + 1, i, xa_next)
                    xp = jnp.concatenate([xa_next, jnp.zeros((SUB - BQ, D), BF16)], axis=0)
                    st = _nt(_unpack(zt_ref[pl.ds((b + 1) * NT // 2, NT // 2), :]), xp)
                    st_ref[(b + 1) * NQ + i, pl.ds(0, BQ), :] = tail_scores(st)[:BQ]

        if not last:
            hooks = {1: startup1, 3: startup3, 4: startup4} if first else {}
            kb = k_ref.at[b if (static or b + 1 == B) else (i + 1) // NQ]
            mms = []
            for sb in range(NSUB):
                if sb in hooks:
                    hooks[sb]()
                if first and sb == G0_AT:
                    state["prev"] = mms[-1][:G]
                    gate_conv()
                qs = q_ref[s + 1, pl.ds(0, HQ), :]
                if sb >= QLINK:
                    qs = link_packed(qs, mms[sb - QLINK])
                elif pvs:
                    qs = link_packed(qs, pvs[NSUB - QLINK + sb])
                if first:
                    sc = _nt(_unpack(jnp.concatenate([qs, zt_ref[pl.ds(0, NT // 2), :]], axis=0)),
                             _cat(kb, sb * SUB, SUB))
                    str_ref[:, sb * SUB:(sb + 1) * SUB] = sc[BQ:]
                    sc = sc[:BQ]
                    for tb in TSCHED.get(sb, ()):
                        st = tail_scores(str_ref[:, tb * SUB:(tb + 1) * SUB])
                        r = tb * SUB
                        while r < min((tb + 1) * SUB, T):
                            n = min((tb + 1) * SUB, (r // BQ + 1) * BQ) - r
                            st_ref[r // BQ, pl.ds(r % BQ, n), :] = st[r - tb * SUB:r - tb * SUB + n]
                            r += n
                    if sb == NSUB - 1:
                        col = jax.lax.broadcasted_iota(jnp.int32, (BQ, 128), 1)
                        tail = jnp.where(col < NT, sc[:, SUB - 128:], NEG)
                        sc = jnp.concatenate([sc[:, :SUB - 128], tail], axis=1)
                elif sb == NSUB - 1:
                    qb = _unpack(qs)
                    k3 = _cat(kb, sb * SUB + 256, 128)
                    sc = jnp.concatenate([_nt(qb, _cat(kb, sb * SUB, 256)),
                                          jnp.concatenate([_nt(qb[:208], k3), _nt(qb[208:], k3)], axis=0),
                                          st_ref[s + 1, pl.ds(0, BQ), :]], axis=1)
                else:
                    sc = _nt(_unpack(qs), _cat(kb, sb * SUB, SUB))
                s_ref[:, sb * SUB:(sb + 1) * SUB] = sc
                mx = sc[:, 0:128] if sb == 0 else jnp.maximum(mms[-1], sc[:, 0:128])
                for t in range(1, SUB // 128):
                    mx = jnp.maximum(mx, sc[:, t * 128:(t + 1) * 128])
                mms.append(mx)
                if sb == 0 and not first:
                    push_block(gm_ref, gm0_ref, mm(normalized(acc_ref[...]), W_VO), i != 0)
                    state["prev"] = None
                    merge_conv((0, 1))
            mx_ref[pl.ds(0, BQ), :] = jnp.broadcast_to(jnp.max(mms[-1], axis=1, keepdims=True), (BQ, 128))
            if first:
                startup_end()
                return carry
            res = x_ref[s, pl.ds(0, BQ), :].astype(F32) + mm(_catb(mc_ref, 0, BQ, (2, 3, 0, 1)), W_ML, W_MG)
            o_ref[s, pl.ds(0, BQ), :] = res.astype(BF16)
            if b == 0:
                @pl.when(i == 0)
                def _():
                    out_copy(0, 16, BQ - 16).start()

                @pl.when(i > 0)
                def _():
                    out_copy(i).start()
            else:
                out_copy(s).start()
            return carry

        for ct in range(2):
            gm2_ref[ct, pl.ds(0, 32), :] = gm_ref[ct, pl.ds(BQ - 16, 32), :]

        def glob_rows(ra, rb):
            glob = mm(normalized(acc_ref[pl.ds(ra, rb - ra), :]), W_VO)
            for ct in range(2):
                gt = glob[:, ct * 128:(ct + 1) * 128]
                d0 = 0 if ra == 0 else ra + 16
                full = jnp.concatenate([gm2_ref[ct, pl.ds(d0, 32 + ra - d0), :], gt]
                                       + ([jnp.zeros((16, 128), F32)] if rb == BQ else []), axis=0)
                gm2_ref[ct, pl.ds(32 + ra, rb - ra), :] = gt
                gm2_ref[2 + ct, pl.ds(d0, full.shape[0] - 16), :] = full[:-16] - full[16:]

        pre_ref[...] = x_ref[s].astype(F32) + mm(_catb(mc_ref, 0, BP, (2, 3)), W_ML)
        glob_rows(0, r1)
        hist = []
        for sb in range(NSUB):
            hist.append(pv_acc(r1, BQ, sb, [hist[-2]] if sb >= 2 else []))
        glob_rows(r1, BQ)
        for ja, jb in zip(ESPLIT[:-1], ESPLIT[1:]):
            rows = [[], []]
            for j in range(ja, jb, 2):
                for ct in range(2):
                    rows[ct].extend(conv_pair(gm2_ref, ct, ct, 16 + j * G, None, None, next_zero()))
            lhs = jnp.concatenate([jnp.concatenate(r, axis=0) for r in rows], axis=1).astype(BF16)
            oa, n = ja * G, (jb - ja) * G
            o_ref[s, pl.ds(oa, n), :] = (pre_ref[pl.ds(oa, n), :] + mm(lhs, W_MG)).astype(BF16)
            out_copy(s, oa, n).start()
        return carry

    block(0, -1)
    wait(3)
    jax.lax.fori_loop(0, NQ, functools.partial(block, 0), 0)
    jax.lax.fori_loop(0, NQ - 1, functools.partial(block, 1), 0)
    block(B - 1, NQ - 1)
    pltpu.make_async_copy(out_hbm, out_hbm, sem_out.at[0]).wait()


@jax.jit
def pallas_standalone__conformer_family_e_branchformer__speech_kernel(x, w_qkv, w_att_out, w_mlp_in, dw_csgu, w_mlp_out, dw_merge, w_merge):
    ws = (w_qkv, w_att_out, w_mlp_in, dw_csgu, w_mlp_out, dw_merge, w_merge)
    out = pl.pallas_call(
        _kernel,
        out_shape=jax.ShapeDtypeStruct((B * T, D), BF16),
        in_specs=[pl.BlockSpec(memory_space=pl.ANY)] * 8,
        out_specs=pl.BlockSpec(memory_space=pl.ANY),
        scratch_shapes=[pltpu.VMEM(w.shape, w.dtype) for w in ws] + [
            pltpu.VMEM((NS, BP, D), BF16),
            pltpu.VMEM((NS + 1, 2, BP, 128), BF16),
            pltpu.VMEM((B, 2, TKP // 2, 128), U32),
            pltpu.VMEM((2, TKP // 2, 128), U32),
            pltpu.VMEM((2, TKP // 2, 128), U32),
            pltpu.VMEM((NS, BP // 2, D), U32),
            pltpu.VMEM((BQ, TKP), F32),
            pltpu.VMEM((BP, 128), F32),
            pltpu.VMEM((BQ, D), F32),
            pltpu.VMEM((BP, D), F32),
            pltpu.VMEM((4, BQ + 32, 128), F32),
            pltpu.VMEM((2, 16, 128), F32),
            pltpu.VMEM((2, BP, 128), F32),
            pltpu.VMEM((4, BQ + 32, 128), F32),
            pltpu.VMEM((2, 48, 128), F32),
            pltpu.VMEM((4, BQ + 32, 128), F32),
            pltpu.VMEM((2, 48, 128), F32),
            pltpu.VMEM((4, BQ + 48, 128), F32),
            pltpu.VMEM((B * NT, D), BF16),
            pltpu.VMEM((B * NT // 2, D), U32),
            pltpu.VMEM((NT, TKP), F32),
            pltpu.VMEM((NS, BP, 128), F32),
            pltpu.VMEM((6, 2 * KT, 8, 128), F32),
            pltpu.VMEM((7, D // 2, D), U32),
            pltpu.VMEM((2, BP, 128), BF16),
            pltpu.VMEM((4, BP, 128), BF16),
            pltpu.VMEM((6, BP, 128), BF16),
            pltpu.VMEM((NS, BP, D), BF16),
            pltpu.SMEM((NZ,), jnp.int32),
            pltpu.SemaphoreType.DMA((5,)),
            pltpu.SemaphoreType.DMA((1,)),
        ],
        compiler_params=pltpu.CompilerParams(vmem_limit_bytes=100 * 1024 * 1024),
    )(x.reshape(B * T, D), *ws)
    return out.reshape(B, T, D)
```

```python
import functools
import math

import jax
import jax.numpy as jnp
import jax.experimental.pallas as pl
import jax.experimental.pallas.tpu as pltpu

F32 = jnp.float32
BF16 = jnp.bfloat16
U32 = jnp.uint32

B, T, D, KT = 2, 4000, 256, 31
HALO = KT // 2
BQ = 400
HQ = BQ // 2
NQ = T // BQ
NS = B * NQ
TKP = 4096
NT = T % 128
SUB = 512
NSUB = TKP // SUB
G = 16
NP = BQ // G
BP = BQ + 16
NZ = 32
EPS = 1e-5
NEG = -1e30
LOG2E = math.log2(math.e)
GELU_C = math.sqrt(2.0 / math.pi)
NT_DIMS = (((1,), (1,)), ((), ()))
QLINK = 2
LN_AT = 1
QP_AT = 4
C1 = 6
G0_AT = 5
TSCHED = {1: (0,), 3: (1, 2), 4: (3, 4), 5: (5,), 6: (6,), 7: (7,)}
RSPLIT = 272
ESPLIT = (0, 16, 26)


def _pack(v):
    return pltpu.bitcast(v, U32)


def _unpack(v):
    return pltpu.bitcast(v, BF16)


def _nt(a, b):
    return jax.lax.dot_general(a, b, NT_DIMS, preferred_element_type=F32)


def _cat(ref, r0, n):
    return _unpack(jnp.concatenate([ref[t, pl.ds(r0 // 2, n // 2), :] for t in range(2)], axis=1))


def _catb(ref, r0, n, tiles=(0, 1)):
    return jnp.concatenate([ref[t, pl.ds(r0, n), :] for t in tiles], axis=1)


def _ln(v, eps):
    mu = jnp.mean(v, axis=-1, keepdims=True)
    c = v - mu
    var = jnp.mean(c * c, axis=-1, keepdims=True)
    return c * jnp.exp2(jnp.log(var + eps) * (-0.5 * LOG2E))


def _gelu2(h):
    z = h * ((h * h) * (GELU_C * 0.044715) + GELU_C)
    return h + h * jnp.tanh(z)


def _where(cond, a, b):
    if isinstance(cond, bool):
        return a if cond else jnp.full_like(a, b)
    return jnp.where(cond, a, b)


def _kernel(x_hbm, wqkv_hbm, wao_hbm, win_hbm, dwc_hbm, wout_hbm, dwm_hbm, wmg_hbm,
            out_hbm,
            wqkv_ref, wao_ref, win_ref, dwc_ref, wout_ref, dwm_ref, wmg_ref,
            x_ref, xl_ref, k_ref, v0_ref, v1_ref, q_ref, s_ref, mx_ref, acc_ref, pre_ref,
            gwin_ref, ghead_ref, u_ref, gm_ref, gm0_ref, lm_ref, lm0_ref, gm2_ref,
            xt_ref, zt_ref, str_ref, st_ref, cw_ref, wp_ref, ugc_ref, mc_ref, tmp_ref, o_ref, zero_ref,
            sem_in, sem_out):
    v_refs = (v0_ref, v1_ref)
    W_A, W_VO, W_U, W_G, W_OUT, W_MG, W_ML = range(7)

    def mm(lhs, *ws):
        w = jnp.concatenate([wp_ref[k] for k in ws], axis=0)
        return jnp.dot(lhs, _unpack(w), preferred_element_type=F32)

    def x_pair(c):
        if c == 0:
            return x_hbm.at[pl.ds(0, BQ), :], x_ref.at[0, pl.ds(16, BQ), :]
        return x_hbm.at[pl.ds(c * BQ - 16, BP), :], x_ref.at[c]

    def out_copy(c, r0=0, n=BQ):
        dst = c * BQ - 16 + r0
        if not isinstance(dst, int):
            dst = pl.multiple_of(dst, 16)
        return pltpu.make_async_copy(o_ref.at[c, pl.ds(r0, n), :], out_hbm.at[pl.ds(dst, n), :], sem_out.at[0])

    w_pairs = [(wqkv_hbm.at[:, pl.ds(0, 2 * D)], wqkv_ref.at[:, pl.ds(0, 2 * D)]),
               (dwc_hbm, dwc_ref), (dwm_hbm, dwm_ref), (win_hbm, win_ref),
               (wqkv_hbm.at[:, pl.ds(2 * D, D)], wqkv_ref.at[:, pl.ds(2 * D, D)]),
               (wao_hbm, wao_ref), (wout_hbm, wout_ref), (wmg_hbm, wmg_ref)]
    t_pairs = [(x_hbm.at[pl.ds((b + 1) * T - NT, NT), :], xt_ref.at[pl.ds(b * NT, NT), :]) for b in range(B)]
    groups = [[w_pairs[0], x_pair(0), x_pair(1)] + t_pairs,
              [x_pair(2), w_pairs[3]] + [x_pair(c) for c in range(3, C1)],
              [x_pair(c) for c in range(C1, NQ)] + w_pairs[4:],
              [x_pair(c) for c in range(NQ, NS)],
              [w_pairs[1], w_pairs[2]]]
    groups = [[pltpu.make_async_copy(src, dst, sem_in.at[k]) for src, dst in grp] for k, grp in enumerate(groups)]

    def start(k):
        for c in groups[k]:
            c.start()

    def wait(k):
        for c in groups[k]:
            c.wait()

    def ln_chunk(b, i, link=None):
        c = b * NQ + i
        h0 = i * HQ if isinstance(i, int) else pl.multiple_of(i * HQ, 8)
        xv = x_ref[c, pl.ds(16, BQ), :]
        if link is not None:
            xv = link(xv)
        xa = _ln(xv.astype(F32), EPS)
        for ct in range(2):
            xt = xa[:, ct * 128:(ct + 1) * 128].astype(BF16)
            xl_ref[c, ct, pl.ds(BQ - 16, 16), :] = xt[:16]
            xl_ref[c + 1, ct, pl.ds(0, BQ - 16), :] = xt[16:]
        lo, hi = [jnp.concatenate([_pack(xl_ref[c, ct, pl.ds(BQ - 16, 16), :]),
                                   _pack(xl_ref[c + 1, ct, pl.ds(0, BQ - 16), :])], axis=0) for ct in range(2)]
        col = jax.lax.broadcasted_iota(jnp.int32, (HQ, 128), 1)
        k_ref[b, 0, pl.ds(h0, HQ), :] = lo
        k_ref[b, 1, pl.ds(h0, HQ), :] = hi
        v_refs[b][0, pl.ds(h0, HQ), :] = lo
        v_refs[b][1, pl.ds(h0, HQ), :] = jnp.where(col == 127, jnp.uint32(0x3F803F80), hi)
        return _unpack(jnp.concatenate([lo, hi], axis=1))

    def repack(v, slot=0):
        n = v.shape[0]
        for ct in range(2):
            tmp_ref[2 * slot + ct, pl.ds(0, n), :] = v[:, ct * 128:(ct + 1) * 128].astype(BF16)
        return _pack(_catb(tmp_ref, 0, n, (2 * slot, 2 * slot + 1)))

    def q_proj(b, i, xa=None):
        if xa is None:
            xa = _cat(k_ref.at[b], i * BQ, BQ)
        q_ref[b * NQ + i, pl.ds(0, HQ), :] = repack(mm(xa, W_A), i % 2 if isinstance(i, int) else 0)

    def tail_scores(st):
        n = st.shape[1]
        return jnp.transpose(jnp.concatenate([st, jnp.full((128 - NT, n), NEG, F32)], axis=0))

    def local_lhs(n):
        v = _catb(xl_ref.at[n + 1], 0, BQ)
        if isinstance(n, int) and n == 0:
            v = jnp.concatenate([_catb(xl_ref.at[0], BQ - 16, 16), v], axis=0)
        return v

    def local_u(n):
        return _gelu2(mm(local_lhs(n), W_U))

    def local_g(n):
        return _ln(_gelu2(mm(local_lhs(n), W_G)), 4.0 * EPS)

    def taps_sum(acc, src_ref, st, wt, w0, n, p0, link, zw):
        for k in range(n):
            wk_ = cw_ref[wt, zw + (w0 + k)]
            wk_ = jnp.concatenate([wk_] * (G // 8), axis=0)
            t = src_ref[st, pl.ds(p0 + k, G), :] * wk_
            if acc is None:
                acc = t if link is None else jnp.where(link[0], link[1], t)
            else:
                acc = acc + t
        return acc

    def conv_pair(src_ref, st, wt, c, mask, prev, zw, scale=None):
        p = taps_sum(None, src_ref, st, wt, KT, G, c + 1, None if prev is None else (mask, prev), zw)
        y0 = taps_sum(p, src_ref, 2 + st, wt, 0, G, c - HALO, None, zw)
        if scale is not None:
            y0 = y0 * scale[:G]
        p1 = p if mask is None else jnp.where(mask, y0, p)
        y1 = taps_sum(p1, src_ref, 2 + st, wt, KT + G, KT - G, c + 1, None, zw)
        if scale is not None:
            y1 = y1 * scale[G:]
        return y0, y1

    def normalized(acc):
        l = acc[:, D - 1:D]
        r = pl.reciprocal(l, approx=True)
        r = r * (2.0 - l * r)
        return (acc * r).astype(BF16)

    def push_block(win, win0, val, joined):
        for ct in range(2):
            new = val[:, ct * 128:(ct + 1) * 128]
            win0[ct, pl.ds(0, 32), :] = win[ct, pl.ds(BQ - 16, 32), :]
            tail = _where(joined, win[ct, pl.ds(BQ, 16), :], 0.0)
            win[ct, pl.ds(0, 16), :] = tail
            win[ct, pl.ds(16, BQ), :] = new
            win[2 + ct, pl.ds(0, BQ), :] = jnp.concatenate([tail, new[:BQ - 16]], axis=0) - new
            win0[ct, pl.ds(32, 16), :] = _where(joined, new[:16], 0.0)

    def startup0():
        start(4)
        start(0)

        def clear(k, carry):
            zero_ref[k] = 0
            return carry
        jax.lax.fori_loop(0, NZ, clear, 0)
        x_ref[0, pl.ds(0, 16), :] = jnp.zeros((16, D), BF16)
        pad = jnp.zeros(((TKP - T) // 2, 128), U32)
        for ct in range(2):
            gwin_ref[ct, pl.ds(0, 16), :] = jnp.zeros((16, 128), F32)
            for r in (gm_ref, lm_ref):
                r[ct, pl.ds(BQ - 16, 48), :] = jnp.zeros((48, 128), F32)
            gm2_ref[ct, pl.ds(BQ + 32, 16), :] = jnp.zeros((16, 128), F32)
            xl_ref[NS, ct, pl.ds(BQ - 16, 16), :] = jnp.zeros((16, 128), BF16)
            for b in range(B):
                k_ref[b, ct, pl.ds(T // 2, (TKP - T) // 2), :] = pad
                v_refs[b][ct, pl.ds(T // 2, (TKP - T) // 2), :] = pad
        wait(4)
        dwm = dwm_ref[...].astype(F32)
        dwc = dwc_ref[...].astype(F32) * 0.5
        for wt in range(6):
            src = dwm if wt < 4 else dwc
            taps = [jnp.broadcast_to(src[k:k + 1, (wt % 4) * 128:(wt % 4 + 1) * 128], (8, 128)) for k in range(KT)]
            if wt < 4:
                taps[HALO] = taps[HALO] + 1.0
            for k in range(KT):
                cw_ref[wt, k] = taps[k]
            for k in range(G):
                cw_ref[wt, KT + k] = taps[k] + taps[G + k] if G + k < KT else taps[k]
            for k in range(KT - G):
                cw_ref[wt, KT + G + k] = -taps[G + k]
        start(1)
        wait(0)
        a = _nt(wqkv_ref[:, 0:D], wqkv_ref[:, D:2 * D])
        wp_ref[W_A] = repack(a * (D ** -0.5 * LOG2E), 1)
        q_proj(0, 0, ln_chunk(0, 0))
        kt = _ln(xt_ref[...].astype(F32), EPS).astype(BF16)
        zt_ref[...] = repack(_nt(kt, _unpack(wp_ref[W_A])), 2)
        ln_chunk(0, 1)

    def startup1():
        wait(1)
        start(2)
        q_proj(0, 1)
        wp_ref[W_U] = _pack(win_ref[:, 0:D])
        wp_ref[W_G] = _pack(win_ref[:, D:2 * D])
        u0 = local_u(0)
        g0 = local_g(0)
        for ct in range(2):
            gt = g0[:, ct * 128:(ct + 1) * 128]
            u_ref[ct] = u0[:, ct * 128:(ct + 1) * 128]
            gwin_ref[ct, pl.ds(16, BP), :] = gt
            gwin_ref[2 + ct, pl.ds(0, BQ), :] = (
                jnp.concatenate([jnp.zeros((16, 128), F32), gt[:BQ - 16]], axis=0) - gt[:BQ])
            ghead_ref[ct] = gt[BQ:]
        for c in range(2, C1):
            ln_chunk(0, c)
        for c in range(2, C1 - 1):
            q_proj(0, c)

    def startup3():
        wait(2)
        start(3)
        q_proj(0, C1 - 1)
        wp_ref[W_OUT] = _pack(wout_ref[...])
        wp_ref[W_MG] = _pack(wmg_ref[0:D, :])
        wp_ref[W_ML] = _pack(wmg_ref[D:2 * D, :])
        for c in range(C1, NQ):
            ln_chunk(0, c)

    def startup4():
        for c in range(C1, NQ - 1):
            q_proj(0, c)

    def startup_end():
        q_proj(0, NQ - 1)
        wvo = jnp.dot(wqkv_ref[:, 2 * D:3 * D], wao_ref[...], preferred_element_type=F32)
        wp_ref[W_VO] = repack(wvo - wvo[D - 1:D, :], 2)

    def block(b, i, carry=None):
        static = isinstance(i, int)
        s = b * NQ + i
        first = static and s < 0
        last = static and s == NS - 1
        if first:
            startup0()

        zero = zero_ref[0]
        zoff = pl.multiple_of(zero, 32)
        negs = -(jax.lax.broadcasted_iota(jnp.int32, (8, 128), 0) + zero) - 1
        state = {"prev": None, "n": 0}

        def never(rows):
            return jnp.concatenate([negs] * (rows // 8), axis=0) >= 0

        def link_packed(v, dep):
            nv = never(HQ)
            du = _pack(dep)
            return jnp.concatenate([jnp.where(nv, du[:HQ], v[:, :128]),
                                    jnp.where(nv, du[HQ:], v[:, 128:])], axis=1)

        never_g = never(G)

        def next_zero():
            state["n"] += 1
            return zero_ref[(state["n"] - 1) % NZ]

        def chain(src_ref, st, wt, c, scale=None):
            link = None if state["prev"] is None else (never_g, state["prev"])
            acc = taps_sum(None, src_ref, st, wt, 0, KT, zoff + (c - HALO), link, next_zero())
            if scale is not None:
                acc = acc * scale
            state["prev"] = acc
            return acc

        def chain2(src_ref, st, wt, c, scale=None):
            y0, y1 = conv_pair(src_ref, st, wt, zoff + c, never_g, state["prev"], next_zero(), scale)
            state["prev"] = y1
            return jnp.concatenate([y0, y1], axis=0)

        def merge_conv(cts, n=NP):
            for ct in cts:
                win, win0 = (gm_ref, gm0_ref) if ct < 2 else (lm_ref, lm0_ref)
                mc_ref[ct, pl.ds(0, G), :] = chain(win0, ct % 2, ct, 16).astype(BF16)
                for j in range(1, NP, 2):
                    mc_ref[ct, pl.ds(j * G, 2 * G), :] = chain2(win, ct % 2, ct, j * G).astype(BF16)
                if n > NP:
                    mc_ref[ct, pl.ds(NP * G, G), :] = chain(win, ct % 2, ct, NP * G).astype(BF16)

        def gate_conv():
            for ct in range(2):
                for j in range(0, NP, 2):
                    n = G if j == NP - 1 else 2 * G
                    acc = (chain if j == NP - 1 else chain2)(gwin_ref, ct, 4 + ct, 16 + j * G,
                                                             u_ref[ct, pl.ds(j * G, n), :])
                    ugc_ref[ct, pl.ds(j * G, n), :] = acc.astype(BF16)

        def pv_acc(r0, r1, sb, dep):
            mxs = mx_ref[pl.ds(r0, r1 - r0), :]
            for d in dep:
                mxs = jnp.where(never(r1 - r0), d, mxs)
            p = jnp.exp2(s_ref[pl.ds(r0, r1 - r0), sb * SUB:(sb + 1) * SUB]
                         - jnp.concatenate([mxs] * (SUB // 128), axis=1))
            pv = jnp.dot(p.astype(BF16), _cat(v_refs[b], sb * SUB, SUB), preferred_element_type=F32)
            if sb == 0:
                acc_ref[pl.ds(r0, r1 - r0), :] = pv
            else:
                acc_ref[pl.ds(r0, r1 - r0), :] += pv
            return pv[:, :128]

        pvs = []
        if not first:
            r1 = RSPLIT if last else BQ
            dep = []
            if not last:
                u = local_u(s + 1)
                for ct in range(2):
                    u_ref[ct, pl.ds(0, 16), :] = u_ref[ct, pl.ds(BQ, 16), :]
                    u_ref[ct, pl.ds(16, BQ), :] = u[:, ct * 128:(ct + 1) * 128]
                g = local_g(s + 1)
                for ct in range(2):
                    gt = g[:, ct * 128:(ct + 1) * 128]
                    full = jnp.concatenate([_where(i != NQ - 1, gwin_ref[ct, pl.ds(BQ, 16), :], 0.0),
                                            ghead_ref[ct], gt[:BQ - 16]], axis=0)
                    gwin_ref[ct, pl.ds(0, BP), :] = full
                    gwin_ref[2 + ct, pl.ds(0, BQ), :] = full[:BQ] - full[16:]
                    gwin_ref[ct, pl.ds(BP, 16), :] = _where(i != NQ - 2, gt[BQ - 16:], 0.0)
                    ghead_ref[ct] = gt[BQ - 16:]
                dep = [u[:, :128], u[:, 128:], g[:, :128], g[:, 128:]]
            push_block(lm_ref, lm0_ref, mm(_catb(ugc_ref, 0, BQ), W_OUT), i != 0)
            merge_conv((2, 3), NP + 1 if last else NP)
            if not last:
                gate_conv()
            xa_next = None
            for sb in range(NSUB):
                pvs.append(pv_acc(0, r1, sb, dep))
                dep = [pvs[sb]]
                if sb == LN_AT and b + 1 < B:
                    lnk = pvs[sb]
                    xa_next = ln_chunk(b + 1, i, lambda xv: _unpack(link_packed(_pack(xv), lnk)))
                if sb == QP_AT and b + 1 < B:
                    q_proj(b + 1, i, xa_next)
                    xp = jnp.concatenate([xa_next, jnp.zeros((SUB - BQ, D), BF16)], axis=0)
                    st = _nt(_unpack(zt_ref[pl.ds((b + 1) * NT // 2, NT // 2), :]), xp)
                    st_ref[(b + 1) * NQ + i, pl.ds(0, BQ), :] = tail_scores(st)[:BQ]

        if not last:
            hooks = {1: startup1, 3: startup3, 4: startup4} if first else {}
            kb = k_ref.at[b if (static or b + 1 == B) else (i + 1) // NQ]
            mms = []
            for sb in range(NSUB):
                if sb in hooks:
                    hooks[sb]()
                if first and sb == G0_AT:
                    state["prev"] = mms[-1][:G]
                    gate_conv()
                qs = q_ref[s + 1, pl.ds(0, HQ), :]
                if sb >= QLINK:
                    qs = link_packed(qs, mms[sb - QLINK])
                elif pvs:
                    qs = link_packed(qs, pvs[NSUB - QLINK + sb])
                if first:
                    zt = zt_ref[pl.ds(0, NT // 2), :]
                    qs = jnp.concatenate([qs, zt], axis=0)
                qb = _unpack(qs)
                if sb == NSUB - 1:
                    k3 = _cat(kb, sb * SUB + 256, 128)
                    sc = jnp.concatenate([_nt(qb, _cat(kb, sb * SUB, 256)),
                                          jnp.concatenate([_nt(qb[:208], k3), _nt(qb[208:], k3)], axis=0)], axis=1)
                else:
                    sc = _nt(qb, _cat(kb, sb * SUB, SUB))
                if first:
                    str_ref[:, sb * SUB:sb * SUB + sc.shape[1]] = sc[BQ:]
                    if sb == NSUB - 1:
                        str_ref[:, TKP - 128:] = _nt(_unpack(zt), _cat(kb, TKP - 128, 128))
                    sc = sc[:BQ]
                if sb == NSUB - 1:
                    sc = jnp.concatenate([sc, st_ref[s + 1, pl.ds(0, BQ), :]], axis=1)
                for tb in TSCHED.get(sb, ()) if first else ():
                    st = tail_scores(str_ref[:, tb * SUB:(tb + 1) * SUB])
                    r = tb * SUB
                    while r < min((tb + 1) * SUB, T):
                        n = min((tb + 1) * SUB, (r // BQ + 1) * BQ) - r
                        st_ref[r // BQ, pl.ds(r % BQ, n), :] = st[r - tb * SUB:r - tb * SUB + n]
                        r += n
                s_ref[:, sb * SUB:(sb + 1) * SUB] = sc
                mx = sc[:, 0:128] if sb == 0 else jnp.maximum(mms[-1], sc[:, 0:128])
                for t in range(1, SUB // 128):
                    mx = jnp.maximum(mx, sc[:, t * 128:(t + 1) * 128])
                mms.append(mx)
                if sb == 0 and not first:
                    push_block(gm_ref, gm0_ref, mm(normalized(acc_ref[...]), W_VO), i != 0)
                    state["prev"] = None
                    merge_conv((0, 1))
            mx_ref[pl.ds(0, BQ), :] = jnp.broadcast_to(jnp.max(mms[-1], axis=1, keepdims=True), (BQ, 128))
            if first:
                startup_end()
                return carry
            res = x_ref[s, pl.ds(0, BQ), :].astype(F32) + mm(_catb(mc_ref, 0, BQ, (2, 3, 0, 1)), W_ML, W_MG)
            o_ref[s, pl.ds(0, BQ), :] = res.astype(BF16)
            if b == 0:
                @pl.when(i == 0)
                def _():
                    out_copy(0, 16, BQ - 16).start()

                @pl.when(i > 0)
                def _():
                    out_copy(i).start()
            else:
                out_copy(s).start()
            return carry

        for ct in range(2):
            gm2_ref[ct, pl.ds(0, 32), :] = gm_ref[ct, pl.ds(BQ - 16, 32), :]

        def glob_rows(ra, rb):
            glob = mm(normalized(acc_ref[pl.ds(ra, rb - ra), :]), W_VO)
            for ct in range(2):
                gt = glob[:, ct * 128:(ct + 1) * 128]
                d0 = 0 if ra == 0 else ra + 16
                full = jnp.concatenate([gm2_ref[ct, pl.ds(d0, 32 + ra - d0), :], gt]
                                       + ([jnp.zeros((16, 128), F32)] if rb == BQ else []), axis=0)
                gm2_ref[ct, pl.ds(32 + ra, rb - ra), :] = gt
                gm2_ref[2 + ct, pl.ds(d0, full.shape[0] - 16), :] = full[:-16] - full[16:]

        pre_ref[...] = x_ref[s].astype(F32) + mm(_catb(mc_ref, 0, BP, (2, 3)), W_ML)
        glob_rows(0, r1)
        hist = []
        for sb in range(NSUB):
            hist.append(pv_acc(r1, BQ, sb, [hist[-2]] if sb >= 2 else []))
        glob_rows(r1, BQ)
        for ja, jb in zip(ESPLIT[:-1], ESPLIT[1:]):
            rows = [[], []]
            for j in range(ja, jb, 2):
                for ct in range(2):
                    rows[ct].extend(conv_pair(gm2_ref, ct, ct, 16 + j * G, None, None, next_zero()))
            lhs = jnp.concatenate([jnp.concatenate(r, axis=0) for r in rows], axis=1).astype(BF16)
            oa, n = ja * G, (jb - ja) * G
            o_ref[s, pl.ds(oa, n), :] = (pre_ref[pl.ds(oa, n), :] + mm(lhs, W_MG)).astype(BF16)
            out_copy(s, oa, n).start()
        return carry

    block(0, -1)
    wait(3)
    jax.lax.fori_loop(0, NQ, functools.partial(block, 0), 0)
    jax.lax.fori_loop(0, NQ - 1, functools.partial(block, 1), 0)
    block(B - 1, NQ - 1)
    pltpu.make_async_copy(out_hbm, out_hbm, sem_out.at[0]).wait()


@jax.jit
def pallas_standalone__conformer_family_e_branchformer__speech_kernel(x, w_qkv, w_att_out, w_mlp_in, dw_csgu, w_mlp_out, dw_merge, w_merge):
    ws = (w_qkv, w_att_out, w_mlp_in, dw_csgu, w_mlp_out, dw_merge, w_merge)
    out = pl.pallas_call(
        _kernel,
        out_shape=jax.ShapeDtypeStruct((B * T, D), BF16),
        in_specs=[pl.BlockSpec(memory_space=pl.ANY)] * 8,
        out_specs=pl.BlockSpec(memory_space=pl.ANY),
        scratch_shapes=[pltpu.VMEM(w.shape, w.dtype) for w in ws] + [
            pltpu.VMEM((NS, BP, D), BF16),
            pltpu.VMEM((NS + 1, 2, BP, 128), BF16),
            pltpu.VMEM((B, 2, TKP // 2, 128), U32),
            pltpu.VMEM((2, TKP // 2, 128), U32),
            pltpu.VMEM((2, TKP // 2, 128), U32),
            pltpu.VMEM((NS, BP // 2, D), U32),
            pltpu.VMEM((BQ, TKP), F32),
            pltpu.VMEM((BP, 128), F32),
            pltpu.VMEM((BQ, D), F32),
            pltpu.VMEM((BP, D), F32),
            pltpu.VMEM((4, BQ + 32, 128), F32),
            pltpu.VMEM((2, 16, 128), F32),
            pltpu.VMEM((2, BP, 128), F32),
            pltpu.VMEM((4, BQ + 32, 128), F32),
            pltpu.VMEM((2, 48, 128), F32),
            pltpu.VMEM((4, BQ + 32, 128), F32),
            pltpu.VMEM((2, 48, 128), F32),
            pltpu.VMEM((4, BQ + 48, 128), F32),
            pltpu.VMEM((B * NT, D), BF16),
            pltpu.VMEM((B * NT // 2, D), U32),
            pltpu.VMEM((NT, TKP), F32),
            pltpu.VMEM((NS, BP, 128), F32),
            pltpu.VMEM((6, 2 * KT, 8, 128), F32),
            pltpu.VMEM((7, D // 2, D), U32),
            pltpu.VMEM((2, BP, 128), BF16),
            pltpu.VMEM((4, BP, 128), BF16),
            pltpu.VMEM((6, BP, 128), BF16),
            pltpu.VMEM((NS, BP, D), BF16),
            pltpu.SMEM((NZ,), jnp.int32),
            pltpu.SemaphoreType.DMA((5,)),
            pltpu.SemaphoreType.DMA((1,)),
        ],
        compiler_params=pltpu.CompilerParams(vmem_limit_bytes=100 * 1024 * 1024),
    )(x.reshape(B * T, D), *ws)
    return out.reshape(B, T, D)
```

```python
import functools
import math

import jax
import jax.numpy as jnp
import jax.experimental.pallas as pl
import jax.experimental.pallas.tpu as pltpu

F32 = jnp.float32
BF16 = jnp.bfloat16
U32 = jnp.uint32

B, T, D, KT = 2, 4000, 256, 31
HALO = KT // 2
BQ = 400
HQ = BQ // 2
NQ = T // BQ
NS = B * NQ
TKP = 4096
NT = T % 128
SUB = 512
NSUB = TKP // SUB
PSUB = 256
G = 16
NP = BQ // G
BP = BQ + 16
NZ = 32
EPS = 1e-5
NEG = -1e30
LOG2E = math.log2(math.e)
GELU_C = math.sqrt(2.0 / math.pi)
NT_DIMS = (((1,), (1,)), ((), ()))
QLINK = 2
LN_AT = 3
QP_AT = 9
C1 = 6
G0_AT = 5
TSCHED = {1: (0,), 3: (1, 2), 4: (3, 4), 5: (5,), 6: (6,), 7: (7,)}
RSPLIT = 272
ESPLIT = (0, 16, 26)


def _pack(v):
    return pltpu.bitcast(v, U32)


def _unpack(v):
    return pltpu.bitcast(v, BF16)


def _nt(a, b):
    return jax.lax.dot_general(a, b, NT_DIMS, preferred_element_type=F32)


def _cat(ref, r0, n):
    return _unpack(jnp.concatenate([ref[t, pl.ds(r0 // 2, n // 2), :] for t in range(2)], axis=1))


def _catb(ref, r0, n, tiles=(0, 1)):
    return jnp.concatenate([ref[t, pl.ds(r0, n), :] for t in tiles], axis=1)


def _ln(v, eps):
    mu = jnp.mean(v, axis=-1, keepdims=True)
    c = v - mu
    var = jnp.mean(c * c, axis=-1, keepdims=True)
    return c * jnp.exp2(jnp.log(var + eps) * (-0.5 * LOG2E))


def _gelu2(h):
    z = h * ((h * h) * (GELU_C * 0.044715) + GELU_C)
    return h + h * jnp.tanh(z)


def _where(cond, a, b):
    if isinstance(cond, bool):
        return a if cond else jnp.full_like(a, b)
    return jnp.where(cond, a, b)


def _kernel(x_hbm, wqkv_hbm, wao_hbm, win_hbm, dwc_hbm, wout_hbm, dwm_hbm, wmg_hbm,
            out_hbm,
            wqkv_ref, wao_ref, win_ref, dwc_ref, wout_ref, dwm_ref, wmg_ref,
            x_ref, xl_ref, k_ref, v0_ref, v1_ref, q_ref, s_ref, mx_ref, acc_ref, pre_ref,
            gwin_ref, ghead_ref, u_ref, gm_ref, gm0_ref, lm_ref, lm0_ref, gm2_ref,
            xt_ref, zt_ref, str_ref, st_ref, cw_ref, wp_ref, ugc_ref, mc_ref, tmp_ref, o_ref, zero_ref,
            sem_in, sem_out):
    v_refs = (v0_ref, v1_ref)
    W_A, W_VO, W_U, W_G, W_OUT, W_MG, W_ML = range(7)

    def mm(lhs, *ws):
        w = jnp.concatenate([wp_ref[k] for k in ws], axis=0)
        return jnp.dot(lhs, _unpack(w), preferred_element_type=F32)

    def x_pair(c):
        if c == 0:
            return x_hbm.at[pl.ds(0, BQ), :], x_ref.at[0, pl.ds(16, BQ), :]
        return x_hbm.at[pl.ds(c * BQ - 16, BP), :], x_ref.at[c]

    def out_copy(c, r0=0, n=BQ):
        dst = c * BQ - 16 + r0
        if not isinstance(dst, int):
            dst = pl.multiple_of(dst, 16)
        return pltpu.make_async_copy(o_ref.at[c, pl.ds(r0, n), :], out_hbm.at[pl.ds(dst, n), :], sem_out.at[0])

    w_pairs = [(wqkv_hbm.at[:, pl.ds(0, 2 * D)], wqkv_ref.at[:, pl.ds(0, 2 * D)]),
               (dwc_hbm, dwc_ref), (dwm_hbm, dwm_ref), (win_hbm, win_ref),
               (wqkv_hbm.at[:, pl.ds(2 * D, D)], wqkv_ref.at[:, pl.ds(2 * D, D)]),
               (wao_hbm, wao_ref), (wout_hbm, wout_ref), (wmg_hbm, wmg_ref)]
    t_pairs = [(x_hbm.at[pl.ds((b + 1) * T - NT, NT), :], xt_ref.at[pl.ds(b * NT, NT), :]) for b in range(B)]
    groups = [[w_pairs[0], x_pair(0), x_pair(1)] + t_pairs,
              [x_pair(2), w_pairs[3]] + [x_pair(c) for c in range(3, C1)],
              [x_pair(c) for c in range(C1, NQ)] + w_pairs[4:],
              [x_pair(c) for c in range(NQ, NS)],
              [w_pairs[1], w_pairs[2]]]
    groups = [[pltpu.make_async_copy(src, dst, sem_in.at[k]) for src, dst in grp] for k, grp in enumerate(groups)]

    def start(k):
        for c in groups[k]:
            c.start()

    def wait(k):
        for c in groups[k]:
            c.wait()

    def ln_chunk(b, i, link=None):
        c = b * NQ + i
        h0 = i * HQ if isinstance(i, int) else pl.multiple_of(i * HQ, 8)
        xv = x_ref[c, pl.ds(16, BQ), :]
        if link is not None:
            xv = link(xv)
        xa = _ln(xv.astype(F32), EPS)
        for ct in range(2):
            xt = xa[:, ct * 128:(ct + 1) * 128].astype(BF16)
            xl_ref[c, ct, pl.ds(BQ - 16, 16), :] = xt[:16]
            xl_ref[c + 1, ct, pl.ds(0, BQ - 16), :] = xt[16:]
        lo, hi = [jnp.concatenate([_pack(xl_ref[c, ct, pl.ds(BQ - 16, 16), :]),
                                   _pack(xl_ref[c + 1, ct, pl.ds(0, BQ - 16), :])], axis=0) for ct in range(2)]
        col = jax.lax.broadcasted_iota(jnp.int32, (HQ, 128), 1)
        k_ref[b, 0, pl.ds(h0, HQ), :] = lo
        k_ref[b, 1, pl.ds(h0, HQ), :] = hi
        v_refs[b][0, pl.ds(h0, HQ), :] = lo
        v_refs[b][1, pl.ds(h0, HQ), :] = jnp.where(col == 127, jnp.uint32(0x3F803F80), hi)
        return _unpack(jnp.concatenate([lo, hi], axis=1))

    def repack(v, slot=0):
        n = v.shape[0]
        for ct in range(2):
            tmp_ref[2 * slot + ct, pl.ds(0, n), :] = v[:, ct * 128:(ct + 1) * 128].astype(BF16)
        return _pack(_catb(tmp_ref, 0, n, (2 * slot, 2 * slot + 1)))

    def q_proj(b, i, xa=None):
        if xa is None:
            xa = _cat(k_ref.at[b], i * BQ, BQ)
        q_ref[b * NQ + i, pl.ds(0, HQ), :] = repack(mm(xa, W_A), i % 2 if isinstance(i, int) else 0)

    def tail_scores(st):
        n = st.shape[1]
        return jnp.transpose(jnp.concatenate([st, jnp.full((128 - NT, n), NEG, F32)], axis=0))

    def local_lhs(n):
        v = _catb(xl_ref.at[n + 1], 0, BQ)
        if isinstance(n, int) and n == 0:
            v = jnp.concatenate([_catb(xl_ref.at[0], BQ - 16, 16), v], axis=0)
        return v

    def local_u(n):
        return _gelu2(mm(local_lhs(n), W_U))

    def local_g(n):
        return _ln(_gelu2(mm(local_lhs(n), W_G)), 4.0 * EPS)

    def taps_sum(acc, src_ref, st, wt, w0, n, p0, link, zw):
        for k in range(n):
            wk_ = cw_ref[wt, zw + (w0 + k)]
            wk_ = jnp.concatenate([wk_] * (G // 8), axis=0)
            t = src_ref[st, pl.ds(p0 + k, G), :] * wk_
            if acc is None:
                acc = t if link is None else jnp.where(link[0], link[1], t)
            else:
                acc = acc + t
        return acc

    def conv_pair(src_ref, st, wt, c, mask, prev, zw, scale=None):
        p = taps_sum(None, src_ref, st, wt, KT, G, c + 1, None if prev is None else (mask, prev), zw)
        y0 = taps_sum(p, src_ref, 2 + st, wt, 0, G, c - HALO, None, zw)
        if scale is not None:
            y0 = y0 * scale[:G]
        p1 = p if mask is None else jnp.where(mask, y0, p)
        y1 = taps_sum(p1, src_ref, 2 + st, wt, KT + G, KT - G, c + 1, None, zw)
        if scale is not None:
            y1 = y1 * scale[G:]
        return y0, y1

    def normalized(acc):
        l = acc[:, D - 1:D]
        r = pl.reciprocal(l, approx=True)
        r = r * (2.0 - l * r)
        return (acc * r).astype(BF16)

    def push_block(win, win0, val, joined):
        for ct in range(2):
            new = val[:, ct * 128:(ct + 1) * 128]
            win0[ct, pl.ds(0, 32), :] = win[ct, pl.ds(BQ - 16, 32), :]
            tail = _where(joined, win[ct, pl.ds(BQ, 16), :], 0.0)
            win[ct, pl.ds(0, 16), :] = tail
            win[ct, pl.ds(16, BQ), :] = new
            win[2 + ct, pl.ds(0, BQ), :] = jnp.concatenate([tail, new[:BQ - 16]], axis=0) - new
            win0[ct, pl.ds(32, 16), :] = _where(joined, new[:16], 0.0)

    def startup0():
        start(4)
        start(0)

        def clear(k, carry):
            zero_ref[k] = 0
            return carry
        jax.lax.fori_loop(0, NZ, clear, 0)
        x_ref[0, pl.ds(0, 16), :] = jnp.zeros((16, D), BF16)
        pad = jnp.zeros(((TKP - T) // 2, 128), U32)
        for ct in range(2):
            gwin_ref[ct, pl.ds(0, 16), :] = jnp.zeros((16, 128), F32)
            for r in (gm_ref, lm_ref):
                r[ct, pl.ds(BQ - 16, 48), :] = jnp.zeros((48, 128), F32)
            gm2_ref[ct, pl.ds(BQ + 32, 16), :] = jnp.zeros((16, 128), F32)
            xl_ref[NS, ct, pl.ds(BQ - 16, 16), :] = jnp.zeros((16, 128), BF16)
            for b in range(B):
                k_ref[b, ct, pl.ds(T // 2, (TKP - T) // 2), :] = pad
                v_refs[b][ct, pl.ds(T // 2, (TKP - T) // 2), :] = pad
        wait(4)
        dwm = dwm_ref[...].astype(F32)
        dwc = dwc_ref[...].astype(F32) * 0.5
        for wt in range(6):
            src = dwm if wt < 4 else dwc
            taps = [jnp.broadcast_to(src[k:k + 1, (wt % 4) * 128:(wt % 4 + 1) * 128], (8, 128)) for k in range(KT)]
            if wt < 4:
                taps[HALO] = taps[HALO] + 1.0
            for k in range(KT):
                cw_ref[wt, k] = taps[k]
            for k in range(G):
                cw_ref[wt, KT + k] = taps[k] + taps[G + k] if G + k < KT else taps[k]
            for k in range(KT - G):
                cw_ref[wt, KT + G + k] = -taps[G + k]
        start(1)
        wait(0)
        a = _nt(wqkv_ref[:, 0:D], wqkv_ref[:, D:2 * D])
        wp_ref[W_A] = repack(a * (D ** -0.5 * LOG2E), 1)
        q_proj(0, 0, ln_chunk(0, 0))
        kt = _ln(xt_ref[...].astype(F32), EPS).astype(BF16)
        zt_ref[...] = repack(_nt(kt, _unpack(wp_ref[W_A])), 2)
        ln_chunk(0, 1)

    def startup1():
        wait(1)
        start(2)
        q_proj(0, 1)
        wp_ref[W_U] = _pack(win_ref[:, 0:D])
        wp_ref[W_G] = _pack(win_ref[:, D:2 * D])
        u0 = local_u(0)
        g0 = local_g(0)
        for ct in range(2):
            gt = g0[:, ct * 128:(ct + 1) * 128]
            u_ref[ct] = u0[:, ct * 128:(ct + 1) * 128]
            gwin_ref[ct, pl.ds(16, BP), :] = gt
            gwin_ref[2 + ct, pl.ds(0, BQ), :] = (
                jnp.concatenate([jnp.zeros((16, 128), F32), gt[:BQ - 16]], axis=0) - gt[:BQ])
            ghead_ref[ct] = gt[BQ:]
        for c in range(2, C1):
            ln_chunk(0, c)
        for c in range(2, C1 - 1):
            q_proj(0, c)

    def startup3():
        wait(2)
        start(3)
        q_proj(0, C1 - 1)
        wp_ref[W_OUT] = _pack(wout_ref[...])
        wp_ref[W_MG] = _pack(wmg_ref[0:D, :])
        wp_ref[W_ML] = _pack(wmg_ref[D:2 * D, :])
        for c in range(C1, NQ):
            ln_chunk(0, c)

    def startup4():
        for c in range(C1, NQ - 1):
            q_proj(0, c)

    def startup_end():
        q_proj(0, NQ - 1)
        wvo = jnp.dot(wqkv_ref[:, 2 * D:3 * D], wao_ref[...], preferred_element_type=F32)
        wp_ref[W_VO] = repack(wvo - wvo[D - 1:D, :], 2)

    def block(b, i, carry=None):
        static = isinstance(i, int)
        s = b * NQ + i
        first = static and s < 0
        last = static and s == NS - 1
        if first:
            startup0()

        zero = zero_ref[0]
        zoff = pl.multiple_of(zero, 32)
        negs = -(jax.lax.broadcasted_iota(jnp.int32, (8, 128), 0) + zero) - 1
        state = {"prev": None, "n": 0}

        def never(rows):
            return jnp.concatenate([negs] * (rows // 8), axis=0) >= 0

        def link_packed(v, dep):
            nv = never(HQ)
            du = _pack(dep)
            return jnp.concatenate([jnp.where(nv, du[:HQ], v[:, :128]),
                                    jnp.where(nv, du[HQ:], v[:, 128:])], axis=1)

        never_g = never(G)

        def next_zero():
            state["n"] += 1
            return zero_ref[(state["n"] - 1) % NZ]

        def chain(src_ref, st, wt, c, scale=None):
            link = None if state["prev"] is None else (never_g, state["prev"])
            acc = taps_sum(None, src_ref, st, wt, 0, KT, zoff + (c - HALO), link, next_zero())
            if scale is not None:
                acc = acc * scale
            state["prev"] = acc
            return acc

        def chain2(src_ref, st, wt, c, scale=None):
            y0, y1 = conv_pair(src_ref, st, wt, zoff + c, never_g, state["prev"], next_zero(), scale)
            state["prev"] = y1
            return jnp.concatenate([y0, y1], axis=0)

        def merge_conv(cts, n=NP):
            for ct in cts:
                win, win0 = (gm_ref, gm0_ref) if ct < 2 else (lm_ref, lm0_ref)
                mc_ref[ct, pl.ds(0, G), :] = chain(win0, ct % 2, ct, 16).astype(BF16)
                for j in range(1, NP, 2):
                    mc_ref[ct, pl.ds(j * G, 2 * G), :] = chain2(win, ct % 2, ct, j * G).astype(BF16)
                if n > NP:
                    mc_ref[ct, pl.ds(NP * G, G), :] = chain(win, ct % 2, ct, NP * G).astype(BF16)

        def gate_conv():
            for ct in range(2):
                for j in range(0, NP, 2):
                    n = G if j == NP - 1 else 2 * G
                    acc = (chain if j == NP - 1 else chain2)(gwin_ref, ct, 4 + ct, 16 + j * G,
                                                             u_ref[ct, pl.ds(j * G, n), :])
                    ugc_ref[ct, pl.ds(j * G, n), :] = acc.astype(BF16)

        nk = SUB if last else PSUB

        def pv_acc(r0, r1, sb, dep):
            mxs = mx_ref[pl.ds(r0, r1 - r0), :]
            for d in dep:
                mxs = jnp.where(never(r1 - r0), d, mxs)
            p = jnp.exp2(s_ref[pl.ds(r0, r1 - r0), sb * nk:(sb + 1) * nk]
                         - jnp.concatenate([mxs] * (nk // 128), axis=1))
            pv = jnp.dot(p.astype(BF16), _cat(v_refs[b], sb * nk, nk), preferred_element_type=F32)
            if sb == 0:
                acc_ref[pl.ds(r0, r1 - r0), :] = pv
            else:
                acc_ref[pl.ds(r0, r1 - r0), :] += pv
            return pv[:, :128]

        pvs = []
        if not first:
            r1 = RSPLIT if last else BQ
            dep = []
            if not last:
                u = local_u(s + 1)
                for ct in range(2):
                    u_ref[ct, pl.ds(0, 16), :] = u_ref[ct, pl.ds(BQ, 16), :]
                    u_ref[ct, pl.ds(16, BQ), :] = u[:, ct * 128:(ct + 1) * 128]
                g = local_g(s + 1)
                for ct in range(2):
                    gt = g[:, ct * 128:(ct + 1) * 128]
                    full = jnp.concatenate([_where(i != NQ - 1, gwin_ref[ct, pl.ds(BQ, 16), :], 0.0),
                                            ghead_ref[ct], gt[:BQ - 16]], axis=0)
                    gwin_ref[ct, pl.ds(0, BP), :] = full
                    gwin_ref[2 + ct, pl.ds(0, BQ), :] = full[:BQ] - full[16:]
                    gwin_ref[ct, pl.ds(BP, 16), :] = _where(i != NQ - 2, gt[BQ - 16:], 0.0)
                    ghead_ref[ct] = gt[BQ - 16:]
                dep = [g[:, 128:]]
            push_block(lm_ref, lm0_ref, mm(_catb(ugc_ref, 0, BQ), W_OUT), i != 0)
            merge_conv((2, 3), NP + 1 if last else NP)
            if not last:
                gate_conv()
            xa_next = None
            for sb in range(TKP // nk):
                pvs.append(pv_acc(0, r1, sb, dep))
                dep = [pvs[sb]]
                if sb == LN_AT and b + 1 < B:
                    lnk = pvs[sb]
                    xa_next = ln_chunk(b + 1, i, lambda xv: _unpack(link_packed(_pack(xv), lnk)))
                if sb == QP_AT and b + 1 < B:
                    q_proj(b + 1, i, xa_next)
                    xp = jnp.concatenate([xa_next, jnp.zeros((SUB - BQ, D), BF16)], axis=0)
                    st = _nt(_unpack(zt_ref[pl.ds((b + 1) * NT // 2, NT // 2), :]), xp)
                    st_ref[(b + 1) * NQ + i, pl.ds(0, BQ), :] = tail_scores(st)[:BQ]

        if not last:
            hooks = {1: startup1, 3: startup3, 4: startup4} if first else {}
            kb = k_ref.at[b if (static or b + 1 == B) else (i + 1) // NQ]
            mms = []
            for sb in range(NSUB):
                if sb in hooks:
                    hooks[sb]()
                if first and sb == G0_AT:
                    state["prev"] = mms[-1][:G]
                    gate_conv()
                qs = q_ref[s + 1, pl.ds(0, HQ), :]
                if sb >= QLINK:
                    qs = link_packed(qs, mms[sb - QLINK])
                elif pvs:
                    qs = link_packed(qs, pvs[sb - QLINK])
                if first:
                    zt = zt_ref[pl.ds(0, NT // 2), :]
                    qs = jnp.concatenate([qs, zt], axis=0)
                qb = _unpack(qs)
                if sb == NSUB - 1:
                    k3 = _cat(kb, sb * SUB + 256, 128)
                    sc = jnp.concatenate([_nt(qb, _cat(kb, sb * SUB, 256)),
                                          jnp.concatenate([_nt(qb[:208], k3), _nt(qb[208:], k3)], axis=0)], axis=1)
                else:
                    sc = _nt(qb, _cat(kb, sb * SUB, SUB))
                if first:
                    str_ref[:, sb * SUB:sb * SUB + sc.shape[1]] = sc[BQ:]
                    if sb == NSUB - 1:
                        str_ref[:, TKP - 128:] = _nt(_unpack(zt), _cat(kb, TKP - 128, 128))
                    sc = sc[:BQ]
                if sb == NSUB - 1:
                    sc = jnp.concatenate([sc, st_ref[s + 1, pl.ds(0, BQ), :]], axis=1)
                for tb in TSCHED.get(sb, ()) if first else ():
                    st = tail_scores(str_ref[:, tb * SUB:(tb + 1) * SUB])
                    r = tb * SUB
                    while r < min((tb + 1) * SUB, T):
                        n = min((tb + 1) * SUB, (r // BQ + 1) * BQ) - r
                        st_ref[r // BQ, pl.ds(r % BQ, n), :] = st[r - tb * SUB:r - tb * SUB + n]
                        r += n
                s_ref[:, sb * SUB:(sb + 1) * SUB] = sc
                mx = sc[:, 0:128] if sb == 0 else jnp.maximum(mms[-1], sc[:, 0:128])
                for t in range(1, SUB // 128):
                    mx = jnp.maximum(mx, sc[:, t * 128:(t + 1) * 128])
                mms.append(mx)
                if sb == 0 and not first:
                    push_block(gm_ref, gm0_ref, mm(normalized(acc_ref[...]), W_VO), i != 0)
                    state["prev"] = None
                    merge_conv((0, 1))
            mx_ref[pl.ds(0, BQ), :] = jnp.broadcast_to(jnp.max(mms[-1], axis=1, keepdims=True), (BQ, 128))
            if first:
                startup_end()
                return carry
            res = x_ref[s, pl.ds(0, BQ), :].astype(F32) + mm(_catb(mc_ref, 0, BQ, (2, 3, 0, 1)), W_ML, W_MG)
            o_ref[s, pl.ds(0, BQ), :] = res.astype(BF16)
            if b == 0:
                @pl.when(i == 0)
                def _():
                    out_copy(0, 16, BQ - 16).start()

                @pl.when(i > 0)
                def _():
                    out_copy(i).start()
            else:
                out_copy(s).start()
            return carry

        for ct in range(2):
            gm2_ref[ct, pl.ds(0, 32), :] = gm_ref[ct, pl.ds(BQ - 16, 32), :]

        def glob_rows(ra, rb):
            glob = mm(normalized(acc_ref[pl.ds(ra, rb - ra), :]), W_VO)
            for ct in range(2):
                gt = glob[:, ct * 128:(ct + 1) * 128]
                d0 = 0 if ra == 0 else ra + 16
                full = jnp.concatenate([gm2_ref[ct, pl.ds(d0, 32 + ra - d0), :], gt]
                                       + ([jnp.zeros((16, 128), F32)] if rb == BQ else []), axis=0)
                gm2_ref[ct, pl.ds(32 + ra, rb - ra), :] = gt
                gm2_ref[2 + ct, pl.ds(d0, full.shape[0] - 16), :] = full[:-16] - full[16:]

        pre_ref[...] = x_ref[s].astype(F32) + mm(_catb(mc_ref, 0, BP, (2, 3)), W_ML)
        glob_rows(0, r1)
        hist = []
        for sb in range(NSUB):
            hist.append(pv_acc(r1, BQ, sb, [hist[-2]] if sb >= 2 else []))
        glob_rows(r1, BQ)
        for ja, jb in zip(ESPLIT[:-1], ESPLIT[1:]):
            rows = [[], []]
            for j in range(ja, jb, 2):
                for ct in range(2):
                    rows[ct].extend(conv_pair(gm2_ref, ct, ct, 16 + j * G, None, None, next_zero()))
            lhs = jnp.concatenate([jnp.concatenate(r, axis=0) for r in rows], axis=1).astype(BF16)
            oa, n = ja * G, (jb - ja) * G
            o_ref[s, pl.ds(oa, n), :] = (pre_ref[pl.ds(oa, n), :] + mm(lhs, W_MG)).astype(BF16)
            out_copy(s, oa, n).start()
        return carry

    block(0, -1)
    wait(3)
    jax.lax.fori_loop(0, NQ, functools.partial(block, 0), 0)
    jax.lax.fori_loop(0, NQ - 1, functools.partial(block, 1), 0)
    block(B - 1, NQ - 1)
    pltpu.make_async_copy(out_hbm, out_hbm, sem_out.at[0]).wait()


@jax.jit
def pallas_standalone__conformer_family_e_branchformer__speech_kernel(x, w_qkv, w_att_out, w_mlp_in, dw_csgu, w_mlp_out, dw_merge, w_merge):
    ws = (w_qkv, w_att_out, w_mlp_in, dw_csgu, w_mlp_out, dw_merge, w_merge)
    out = pl.pallas_call(
        _kernel,
        out_shape=jax.ShapeDtypeStruct((B * T, D), BF16),
        in_specs=[pl.BlockSpec(memory_space=pl.ANY)] * 8,
        out_specs=pl.BlockSpec(memory_space=pl.ANY),
        scratch_shapes=[pltpu.VMEM(w.shape, w.dtype) for w in ws] + [
            pltpu.VMEM((NS, BP, D), BF16),
            pltpu.VMEM((NS + 1, 2, BP, 128), BF16),
            pltpu.VMEM((B, 2, TKP // 2, 128), U32),
            pltpu.VMEM((2, TKP // 2, 128), U32),
            pltpu.VMEM((2, TKP // 2, 128), U32),
            pltpu.VMEM((NS, BP // 2, D), U32),
            pltpu.VMEM((BQ, TKP), F32),
            pltpu.VMEM((BP, 128), F32),
            pltpu.VMEM((BQ, D), F32),
            pltpu.VMEM((BP, D), F32),
            pltpu.VMEM((4, BQ + 32, 128), F32),
            pltpu.VMEM((2, 16, 128), F32),
            pltpu.VMEM((2, BP, 128), F32),
            pltpu.VMEM((4, BQ + 32, 128), F32),
            pltpu.VMEM((2, 48, 128), F32),
            pltpu.VMEM((4, BQ + 32, 128), F32),
            pltpu.VMEM((2, 48, 128), F32),
            pltpu.VMEM((4, BQ + 48, 128), F32),
            pltpu.VMEM((B * NT, D), BF16),
            pltpu.VMEM((B * NT // 2, D), U32),
            pltpu.VMEM((NT, TKP), F32),
            pltpu.VMEM((NS, BP, 128), F32),
            pltpu.VMEM((6, 2 * KT, 8, 128), F32),
            pltpu.VMEM((7, D // 2, D), U32),
            pltpu.VMEM((2, BP, 128), BF16),
            pltpu.VMEM((4, BP, 128), BF16),
            pltpu.VMEM((6, BP, 128), BF16),
            pltpu.VMEM((NS, BP, D), BF16),
            pltpu.SMEM((NZ,), jnp.int32),
            pltpu.SemaphoreType.DMA((5,)),
            pltpu.SemaphoreType.DMA((1,)),
        ],
        compiler_params=pltpu.CompilerParams(vmem_limit_bytes=100 * 1024 * 1024),
    )(x.reshape(B * T, D), *ws)
    return out.reshape(B, T, D)
```
